```python
import os as _os
_os.environ.setdefault('JAX_PLATFORMS', 'cpu')
import jax
import jax.numpy as jnp

def _softmax(x, axis=-1):
    return jax.nn.softmax(x, axis=axis)

def _gelu(x):
    return jax.nn.gelu(x, approximate=True)

def _silu(x):
    return jax.nn.silu(x)

def _sigmoid(x):
    return jax.nn.sigmoid(x)

def _layernorm(x, axis=-1, eps=1e-05):
    m = jnp.mean(x, axis=axis, keepdims=True)
    v = jnp.var(x, axis=axis, keepdims=True)
    return (x - m) / jnp.sqrt(v + eps)

def _scatter_add(tgt, idx, src, axis=0):
    return tgt.at[idx].add(src)

def _segment_sum(src, seg, n):
    return jax.ops.segment_sum(src, seg, n)

class _Rng:

    def __init__(self, key):
        self._k = key

    def _next(self):
        self._k, sub = jax.random.split(self._k)
        return sub

    def normal(self, shape):
        return jax.random.normal(self._next(), shape, dtype=jnp.bfloat16)

    def randint(self, lo, hi, shape):
        return jax.random.randint(self._next(), shape, lo, hi, dtype=jnp.int32)

    def uniform(self, shape, lo=0.0, hi=1.0):
        return jax.random.uniform(self._next(), shape, jnp.bfloat16, lo, hi)

    def permutation(self, n):
        return jax.random.permutation(self._next(), n)
kernel_name = 'standalone__conformer_family_e_branchformer__speech'

def setup_inputs():
    _rng = _Rng(jax.random.key(int.from_bytes(__import__("os").urandom(4), "little")))
    _w = lambda a: (lambda t: t.astype(jnp.bfloat16) if jnp.issubdtype(t.dtype, jnp.floating) else t)(jnp.asarray(a))
    B, T, D, K = (2, 4000, 512, 5)
    return {'x': _w((lambda *s: _rng.normal(s) * 0.05)(B, T, D)), 'w_qkv': _w((lambda *s: _rng.normal(s) * 0.05)(D, 3 * D)), 'w_att_out': _w((lambda *s: _rng.normal(s) * 0.05)(D, D)), 'w_mlp_in': _w((lambda *s: _rng.normal(s) * 0.05)(D, 2 * D)), 'dw_csgu': _w((lambda *s: _rng.normal(s) * 0.05)(K, D)), 'w_mlp_out': _w((lambda *s: _rng.normal(s) * 0.05)(D, D)), 'dw_merge': _w((lambda *s: _rng.normal(s) * 0.05)(K, 2 * D)), 'w_merge': _w((lambda *s: _rng.normal(s) * 0.05)(2 * D, D))}

def reference(x, w_qkv, w_att_out, w_mlp_in, dw_csgu, w_mlp_out, dw_merge, w_merge):
    B, T, D = x.shape
    K = dw_csgu.shape[0]
    pad = K // 2
    xa = _layernorm(x, axis=-1)
    qkv = jnp.einsum('btd,de->bte', xa, w_qkv)
    q, k, v = (qkv[..., :D].copy(), qkv[..., D:2 * D].copy(), qkv[..., 2 * D:].copy())
    scores = jnp.einsum('btd,bsd->bts', q, k) * D ** (-0.5)
    p = _softmax(scores, axis=-1)
    attn = jnp.einsum('bts,bsd->btd', p, v)
    glob = jnp.einsum('btd,de->bte', attn, w_att_out)
    xc = _layernorm(x, axis=-1)
    h = _gelu(jnp.einsum('btd,de->bte', xc, w_mlp_in))
    u, g = (h[..., :D].copy(), h[..., D:].copy())
    g = _layernorm(g, axis=-1)
    gp = jnp.pad(g, ((0, 0), (pad, pad), (0, 0)))
    gc = jnp.zeros_like(g)
    for i in range(K):
        gc = gc + gp[:, i:i + T, :] * dw_csgu[i][None, None, :]
    loc = jnp.einsum('btd,de->bte', u * gc, w_mlp_out)
    m = jnp.concatenate([glob, loc], axis=-1)
    mp = jnp.pad(m, ((0, 0), (pad, pad), (0, 0)))
    mc = jnp.zeros_like(m)
    for i in range(K):
        mc = mc + mp[:, i:i + T, :] * dw_merge[i][None, None, :]
    m = m + mc
    return x + jnp.einsum('btc,cd->btd', m, w_merge)
```

```python
import functools
import jax
import jax.numpy as jnp
from jax.experimental import pallas as pl
from jax.experimental.pallas import tpu as pltpu

F32 = jnp.float32
BF16 = jnp.bfloat16
U32 = jnp.uint32
LOG2E = 1.4426950408889634
NT = (((1,), (1,)), ((), ()))
LANES = 128
CFG = dict(CK=512, P2AT=[1, 2, 3], MAT=[4, 6, 8], MB=[0, 144, 272, 400], LB=[0, 144, 272, 400], LNAT=5)


def _ln(x, eps=1e-5):
    m = jnp.mean(x, axis=-1, keepdims=True)
    xc = x - m
    v = jnp.mean(xc * xc, axis=-1, keepdims=True)
    return xc * jax.lax.rsqrt(v + eps)


def _gelu(x):
    c = 0.7978845608028654
    t = x * x
    z = x * (t * (c * 0.044715) + c)
    h = 0.5 * x
    return h * jnp.tanh(z) + h


def _ones_last(xn):
    lane = jax.lax.broadcasted_iota(jnp.int32, xn.shape, 1)
    return jnp.where(lane == LANES - 1, jnp.ones_like(xn), xn)


def _pk(x):
    return pltpu.bitcast(x, U32)


def _upk(x):
    return pltpu.bitcast(x, BF16)


def kernel(x_hbm, wqkv_hbm, wo_hbm, win_hbm, dw1_hbm, wout_hbm, dw2_hbm, wm_hbm, o_hbm,
           x_ref, wqkv_ref, wo_ref, win_ref, dw1_ref, wout_ref, dw2_ref, wm_ref,
           xa_s, v3_s, wqk_s, wvo_s, m_s, g_s, o_s, on_s, loc_s, isem, osem,
           *, B, T, D, TQ, NQ, TP, CK, P, TL, P2AT, MAT, MB, LB, LNAT):
    H = 8
    NC = TP // CK
    NB = B * NQ
    ND = D // LANES
    LAG = 2
    NP = len(LB) - 1
    NM = len(MB) - 1

    names = ['wqk', 'dw1', 'dw2', 'wv', 'wo', 'win', 'wout', 'wm', 'x1']
    pairs = dict(
        wqk=(wqkv_hbm.at[:, 0:2 * D], wqkv_ref.at[:, 0:2 * D]),
        wv=(wqkv_hbm.at[:, 2 * D:3 * D], wqkv_ref.at[:, 2 * D:3 * D]),
        win=(win_hbm, win_ref), dw1=(dw1_hbm, dw1_ref), wout=(wout_hbm, wout_ref), wo=(wo_hbm, wo_ref),
        dw2=(dw2_hbm, dw2_ref), wm=(wm_hbm, wm_ref.at[1]), x1=(x_hbm.at[1], x_ref.at[1]))

    def in_copy(name):
        src, dst = pairs[name]
        return pltpu.make_async_copy(src, dst, isem.at[names.index(name)])

    def x0_copy(j):
        r = pl.multiple_of(j * TQ, 16)
        return pltpu.make_async_copy(x_hbm.at[0, pl.ds(r, TQ), :], x_ref.at[0, pl.ds(r, TQ), :],
                                     isem.at[len(names) + j])

    def out_copy(nm):
        slot = nm % 2
        return pltpu.make_async_copy(
            o_s.at[slot], o_hbm.at[nm // NQ, pl.ds(pl.multiple_of((nm % NQ) * TQ, 16), TQ), :], osem.at[slot])

    for name in names[:5]:
        in_copy(name).start()
    for j in range(NQ):
        x0_copy(j).start()
    for name in names[5:]:
        in_copy(name).start()
    z = jnp.zeros((2 * ND, H, LANES), F32)
    for b in range(B):
        m_s[b, :, 0:H, :] = z
        m_s[b, :, H + T:H + T + H, :] = z
        xa_s[b, 0:P // 2, :] = jnp.zeros((P // 2, D), U32)
        xa_s[b, (P + T) // 2:(P + TP) // 2, :] = jnp.zeros(((TP - T) // 2, D), U32)
        v3_s[b, T // 2:TP // 2, :] = jnp.zeros(((TP - T) // 2, LANES), U32)
    m_s[0, :, H:H + TQ + H, :] = jnp.zeros((2 * ND, TQ + H, LANES), F32)
    on_s[...] = jnp.zeros(on_s.shape, U32)
    loc_s[...] = jnp.zeros(loc_s.shape, F32)
    wm_ref[0] = jnp.zeros(wm_ref.shape[1:], BF16)
    in_copy('wqk').wait()
    wqk_s[...] = _pk((jax.lax.dot_general(wqkv_ref[:, 0:D], wqkv_ref[:, D:2 * D], NT, preferred_element_type=F32)
                      * (D ** -0.5 * LOG2E)).astype(BF16))

    def fold_wvo():
        in_copy('wv').wait()
        in_copy('wo').wait()
        wvo = jnp.dot(wqkv_ref[:, 2 * D:3 * D], wo_ref[...], preferred_element_type=F32)
        wvo_s[...] = _pk((wvo - wvo[D - 1:D, :]).astype(BF16))

    fold_wvo()

    def ln0(j, c):
        r = pl.multiple_of(j * TQ, 16)
        x0_copy(j).wait()
        xn = _ln(x_ref[0, pl.ds(r, TQ), :].astype(F32))
        rh = pl.multiple_of(j * (TQ // 2), 8)
        xa_s[0, pl.ds(P // 2 + rh, TQ // 2), :] = _pk(xn.astype(BF16))
        v3_s[0, pl.ds(rh, TQ // 2), :] = _pk(_ones_last(xn[:, D - LANES:]).astype(BF16))
        return c
    jax.lax.fori_loop(0, NQ, ln0, 0)
    for name in ('dw1', 'dw2', 'win', 'wout'):
        in_copy(name).wait()

    def publish_prev(n):
        npv = jnp.maximum(n - 1, 0)
        rr = pl.multiple_of(H + (npv % NQ) * TQ, 8)
        for j in range(ND):
            m_s[npv // NQ, ND + j, pl.ds(rr, TQ), :] = loc_s[j]
        glob = jnp.dot(_upk(on_s[...]), _upk(wvo_s[...]), preferred_element_type=F32)
        for j in range(ND):
            m_s[npv // NQ, j, pl.ds(rr, TQ), :] = glob[:, j * LANES:(j + 1) * LANES]

    def step(n, do_attn, do_merge, ramp=False):
        def first_use(*ids):
            if ramp:
                @pl.when(n == 0)
                def _():
                    for i in ids:
                        in_copy(i).wait()

        if do_merge:
            nm = jnp.maximum(n - LAG, 0)
            wslot = (n >= LAG).astype(jnp.int32)
            bm = nm // NQ
            rm = pl.multiple_of((nm % NQ) * TQ, 16)

        def merge_piece(i):
            lo, sz = MB[i], MB[i + 1] - MB[i]
            dw2 = dw2_ref[...].astype(F32)
            dw2 = dw2 + (jax.lax.broadcasted_iota(jnp.int32, dw2.shape, 0) == 2).astype(F32)
            tiles = []
            for j in range(2 * ND):
                acc = None
                for k in range(5):
                    t = (m_s[bm, j, pl.ds(rm + (lo + H - 2 + k), sz), :]
                         * dw2[k:k + 1, j * LANES:(j + 1) * LANES])
                    acc = t if acc is None else acc + t
                tiles.append(acc.astype(BF16))
            y = jnp.dot(jnp.concatenate(tiles, axis=1), wm_ref[wslot], preferred_element_type=F32)
            xr = x_ref[bm, pl.ds(rm + lo, sz), :].astype(F32)
            o_s[n % 2, lo:lo + sz, :] = (xr + y).astype(o_s.dtype)

        if not do_attn:
            for i in range(NM):
                merge_piece(i)
            return

        b = n // NQ
        rh = pl.multiple_of((n % NQ) * (TQ // 2), 8)

        def xa_rows(lo, size):
            return _upk(xa_s[b, pl.ds(rh + lo // 2, size // 2), :])

        def ln_lead():
            rl = pl.multiple_of(jnp.clip((n - 1) * TL, 0, T - TL), 16)
            xn = _ln(x_ref[jnp.minimum(n, 1), pl.ds(rl, TL), :].astype(F32))
            rlh = pl.multiple_of(jnp.clip((n - 1) * (TL // 2), 0, (T - TL) // 2), 8)
            xa_s[1, pl.ds(P // 2 + rlh, TL // 2), :] = _pk(xn.astype(BF16))
            v3_s[1, pl.ds(rlh, TL // 2), :] = _pk(_ones_last(xn[:, D - LANES:]).astype(BF16))

        if LNAT < 0:
            ln_lead()
        q = jnp.dot(xa_rows(P, TQ), _upk(wqk_s[...]), preferred_element_type=F32).astype(BF16)
        gb = [0] + [2 * P + LB[i + 1] for i in range(NP - 1)] + [TQ + 2 * P]
        hs = {}

        def loc_proj():
            first_use('win')
            hs['g'] = jnp.dot(xa_rows(0, TQ + 2 * P), win_ref[:, D:2 * D], preferred_element_type=F32)
            hs['u'] = jnp.dot(xa_rows(P, TQ), win_ref[:, 0:D], preferred_element_type=F32)

        def loc_piece(i):
            if i == 0:
                first_use('dw1', 'wout')
            dw1 = dw1_ref[...].astype(F32)
            g = _ln(_gelu(hs['g'][gb[i]:gb[i + 1]]))
            for j in range(ND):
                g_s[j, gb[i]:gb[i + 1], :] = g[:, j * LANES:(j + 1) * LANES]
            u = _gelu(hs['u'][LB[i]:LB[i + 1]])
            tiles = []
            for j in range(ND):
                acc = None
                for k in range(5):
                    lo = P + LB[i] - 2 + k
                    t = g_s[j, lo:lo + LB[i + 1] - LB[i], :] * dw1[k:k + 1, j * LANES:(j + 1) * LANES]
                    acc = t if acc is None else acc + t
                tiles.append((u[:, j * LANES:(j + 1) * LANES] * acc).astype(BF16))
            loc = jnp.dot(jnp.concatenate(tiles, axis=1), wout_ref[...], preferred_element_type=F32)
            for j in range(ND):
                loc_s[j, LB[i]:LB[i + 1], :] = loc[:, j * LANES:(j + 1) * LANES]

        def schunk(c):
            k = _upk(xa_s[b, pl.ds((P + c * CK) // 2, CK // 2), :])
            s = jax.lax.dot_general(q, k, NT, preferred_element_type=F32)
            if (c + 1) * CK > T:
                col = c * CK + jax.lax.broadcasted_iota(jnp.int32, (TQ, CK), 1)
                s = jnp.where(col < T, s, -jnp.inf)
            return s

        def vchunk(lo, size):
            return _upk(jnp.concatenate([xa_s[b, pl.ds((P + lo) // 2, size // 2), 0:D - LANES],
                                         v3_s[b, pl.ds(lo // 2, size // 2), :]], axis=1))

        def rowmax(s):
            t = s[:, 0:128]
            for j in range(1, s.shape[1] // 128):
                t = jnp.maximum(t, s[:, j * 128:(j + 1) * 128])
            return t

        side = [[] for _ in range(NC + 1)]
        for i in range(NP):
            side[P2AT[i]].append(functools.partial(loc_piece, i))
        side[0].append(loc_proj)
        if do_merge:
            for i in range(NM):
                side[MAT[i]].append(functools.partial(merge_piece, i))
        if LNAT >= 0:
            side[LNAT].append(ln_lead)
        mrun = None
        acc = None
        s_next = schunk(0)
        for c in range(NC):
            s = s_next
            if c + 1 < NC:
                s_next = schunk(c + 1)
            mc = jnp.max(rowmax(s), axis=-1, keepdims=True)
            mnew = mc if mrun is None else jnp.maximum(mrun, mc)
            p = jnp.exp2(s - mnew).astype(BF16)
            for task in side[c]:
                task()
            d = jnp.dot(p, vchunk(c * CK, CK), preferred_element_type=F32)
            if mrun is None:
                acc = d
            else:
                acc = acc * jnp.exp2(mrun - mnew) + d
            mrun = mnew
        for task in side[NC]:
            task()
        l = acc[:, D - 1:D]
        on_s[...] = _pk((acc * (1.0 / l)).astype(BF16))

    def pre(n):
        @pl.when(n >= LAG + 2)
        def _():
            out_copy(n - 2 - LAG).wait()

    def post(n):
        @pl.when(n >= LAG)
        def _():
            out_copy(n - LAG).start()

    def main(n, c):
        @pl.when(n == 1)
        def _():
            in_copy('x1').wait()

        @pl.when(n == LAG)
        def _():
            in_copy('wm').wait()
        pre(n)
        publish_prev(n)
        step(n, True, True)
        post(n)
        return c
    jax.lax.fori_loop(0, NB, main, 0)

    pre(jnp.int32(NB))
    publish_prev(jnp.int32(NB))
    step(jnp.int32(NB), False, True)
    post(jnp.int32(NB))
    pre(jnp.int32(NB + 1))
    step(jnp.int32(NB + 1), False, True)
    post(jnp.int32(NB + 1))
    out_copy(NB - 2).wait()
    out_copy(NB - 1).wait()


@jax.jit
def pallas_standalone__conformer_family_e_branchformer__speech_kernel(
    x, w_qkv, w_att_out, w_mlp_in, dw_csgu, w_mlp_out, dw_merge, w_merge):
    B, T, D = x.shape
    TQ = 400
    NQ = T // TQ
    CK = CFG['CK']
    TP = -(-T // CK) * CK
    P = 16
    H = 8
    TL = 448
    assert -(-T // TL) <= NQ - 1
    hbm = pl.BlockSpec(memory_space=pl.ANY)
    ins = (x, w_qkv, w_att_out, w_mlp_in, dw_csgu, w_mlp_out, dw_merge, w_merge)

    return pl.pallas_call(
        functools.partial(kernel, B=B, T=T, D=D, TQ=TQ, NQ=NQ, TP=TP, P=P, TL=TL, **CFG),
        in_specs=[hbm] * len(ins),
        out_specs=hbm,
        out_shape=jax.ShapeDtypeStruct((B, T, D), x.dtype),
        scratch_shapes=[pltpu.VMEM(a.shape, a.dtype) for a in ins[:-1]] + [
            pltpu.VMEM((2,) + w_merge.shape, w_merge.dtype),
            pltpu.VMEM((B, (P + TP) // 2, D), U32),
            pltpu.VMEM((B, TP // 2, LANES), U32),
            pltpu.VMEM((D // 2, D), U32),
            pltpu.VMEM((D // 2, D), U32),
            pltpu.VMEM((B, 2 * D // LANES, T + 2 * H, LANES), F32),
            pltpu.VMEM((D // LANES, TQ + 2 * P, LANES), F32),
            pltpu.VMEM((2, TQ, D), BF16),
            pltpu.VMEM((TQ // 2, D), U32),
            pltpu.VMEM((D // LANES, TQ, LANES), F32),
            pltpu.SemaphoreType.DMA((9 + NQ,)),
            pltpu.SemaphoreType.DMA((2,)),
        ],
        compiler_params=pltpu.CompilerParams(
            vmem_limit_bytes=110 * 1024 * 1024),
    )(x, w_qkv, w_att_out, w_mlp_in, dw_csgu, w_mlp_out, dw_merge, w_merge)
```

```python
import functools
import jax
import jax.numpy as jnp
from jax.experimental import pallas as pl
from jax.experimental.pallas import tpu as pltpu

F32 = jnp.float32
BF16 = jnp.bfloat16
LOG2E = 1.4426950408889634
NT = (((1,), (1,)), ((), ()))
LANES = 128
CFG = dict(CK=512, P2AT=[1, 2, 3, 4], MAT=[8], MB=[0, 400], LB=[0, 96, 208, 304, 400], TL=400,
           TMB=[0, 400], CARRY=1, KC=1, TKC=1, KAT=[4, 5, 5, 6, 6, 7, 7, 8])


def _ln(x, eps=1e-5):
    m = jnp.mean(x, axis=-1, keepdims=True)
    xc = x - m
    v = jnp.mean(xc * xc, axis=-1, keepdims=True)
    return xc * jnp.exp2(jnp.log(v + eps) * (-0.5 * LOG2E))


def _gelu(x):
    c = 0.7978845608028654
    t = x * x
    z = x * (t * (c * 0.044715) + c)
    h = 0.5 * x
    return h * jnp.tanh(z) + h


def _ones_last(xn):
    lane = jax.lax.broadcasted_iota(jnp.int32, xn.shape, 1)
    return jnp.where(lane == LANES - 1, jnp.ones_like(xn), xn)


def kernel(x_hbm, wqkv_hbm, wo_hbm, win_hbm, dw1_hbm, wout_hbm, dw2_hbm, wm_hbm, o_hbm,
           x_ref, wqkv_ref, wo_ref, win_ref, dw1_ref, wout_ref, dw2_ref, wm_ref,
           xa_s, v3_s, wqk_s, wvo_s, w_s, n_s, g_s, o_s, on_s, loc_s, isem, xsem, osem,
           *, B, T, D, TQ, NQ, TP, CK, P, TL, P2AT, MAT, MB, LB, TMB, CARRY, KC, TKC, KAT):
    H = 8
    NC = TP // CK
    NB = B * NQ
    ND = D // LANES
    LAG = 2
    NP = len(LB) - 1
    NM = len(MB) - 1
    NL = T // TL

    names = ['wqk', 'dw1', 'dw2', 'wv', 'wo', 'win', 'wout', 'wm']
    pairs = dict(
        wqk=(wqkv_hbm.at[:, 0:2 * D], wqkv_ref.at[:, 0:2 * D]),
        wv=(wqkv_hbm.at[:, 2 * D:3 * D], wqkv_ref.at[:, 2 * D:3 * D]),
        win=(win_hbm, win_ref), dw1=(dw1_hbm, dw1_ref), wout=(wout_hbm, wout_ref), wo=(wo_hbm, wo_ref),
        dw2=(dw2_hbm, dw2_ref), wm=(wm_hbm, wm_ref.at[1]))

    def in_copy(name):
        src, dst = pairs[name]
        return pltpu.make_async_copy(src, dst, isem.at[names.index(name)])

    XG = [0, 5, 9, 10]

    def x0_copy(g):
        lo, hi = XG[g] * TL, XG[g + 1] * TL
        return pltpu.make_async_copy(x_hbm.at[0, lo:hi, :], x_ref.at[0, lo:hi, :], xsem.at[g])

    def x1_copy():
        return pltpu.make_async_copy(x_hbm.at[1], x_ref.at[1], xsem.at[NL])

    def back(b, i, k):
        wrap = i < k
        bb = jnp.where(wrap, b - 1, b)
        ii = jnp.where(wrap, i + (NQ - k), i - k)
        first = bb < 0
        return jnp.where(first, 0, bb), pl.multiple_of(jnp.where(first, 0, ii) * TQ, 16)

    def out_copy(slot, bb, rr):
        return pltpu.make_async_copy(o_s.at[slot], o_hbm.at[bb, pl.ds(rr, TQ), :], osem.at[slot])

    for name in names[:5]:
        in_copy(name).start()
    for g in range(len(XG) - 2):
        x0_copy(g).start()
    in_copy('win').start()
    x0_copy(len(XG) - 2).start()
    for name in names[6:]:
        in_copy(name).start()
    x1_copy().start()
    xa_s[0:P, :] = jnp.zeros((P, D), BF16)
    xa_s[P + T:, :] = jnp.zeros((xa_s.shape[0] - P - T, D), BF16)
    v3_s[T:TP, :] = jnp.zeros((TP - T, LANES), BF16)
    w_s[...] = jnp.zeros(w_s.shape, F32)
    n_s[...] = jnp.zeros(n_s.shape, F32)
    on_s[...] = jnp.zeros(on_s.shape, BF16)
    loc_s[...] = jnp.zeros(loc_s.shape, F32)
    wm_ref[0] = jnp.zeros(wm_ref.shape[1:], BF16)
    in_copy('wqk').wait()
    wqk_s[...] = (jax.lax.dot_general(wqkv_ref[:, 0:D], wqkv_ref[:, D:2 * D], NT, preferred_element_type=F32)
                  * (D ** -0.5 * LOG2E)).astype(BF16)
    in_copy('wv').wait()
    in_copy('wo').wait()
    wvo = jnp.dot(wqkv_ref[:, 2 * D:3 * D], wo_ref[...], preferred_element_type=F32)
    wvo_s[...] = (wvo - wvo[D - 1:D, :]).astype(BF16)

    def publish_prev():
        for j in range(ND):
            n_s[ND + j, H:H + TQ, :] = loc_s[j]
        glob = jnp.dot(on_s[...], wvo_s[...], preferred_element_type=F32)
        for j in range(ND):
            n_s[j, H:H + TQ, :] = glob[:, j * LANES:(j + 1) * LANES]

    def edge(rows, keep):
        return jnp.where(keep, rows, jnp.zeros_like(rows))

    def top_up(keep):
        w_s[:, H + TQ:H + TQ + H, :] = edge(n_s[:, H:2 * H, :], keep)

    def shift(keep):
        w_s[:, 0:H, :] = edge(w_s[:, TQ:TQ + H, :], keep)
        w_s[:, H:H + TQ, :] = n_s[:, H:H + TQ, :]

    def gate(h):
        return _ln(_gelu(h))

    def merge(win, b, i, slot, bounds, kc):
        bm, rm = back(b, i, LAG)
        wslot = jnp.logical_or(b > 0, i >= LAG).astype(jnp.int32)
        ys = {}

        def piece(k, j0):
            lo, sz = bounds[k], bounds[k + 1] - bounds[k]
            dw2 = dw2_ref[...].astype(F32)
            dw2 = dw2 + (jax.lax.broadcasted_iota(jnp.int32, dw2.shape, 0) == 2).astype(F32)
            tiles = []
            for j in range(j0, j0 + kc):
                acc = None
                for t in range(5):
                    v = (win[j, lo + H - 2 + t:lo + H - 2 + t + sz, :]
                         * dw2[t:t + 1, j * LANES:(j + 1) * LANES])
                    acc = v if acc is None else acc + v
                tiles.append(acc.astype(BF16))
            d = jnp.dot(jnp.concatenate(tiles, axis=1), wm_ref[wslot, j0 * LANES:(j0 + kc) * LANES, :],
                        preferred_element_type=F32)
            ys[k] = d if j0 == 0 else ys[k] + d
            if j0 + kc == 2 * ND:
                xr = x_ref[bm, pl.ds(rm + lo, sz), :].astype(F32)
                o_s[slot, lo:lo + sz, :] = (xr + ys[k]).astype(o_s.dtype)
        return [functools.partial(piece, k, j0) for k in range(len(bounds) - 1) for j0 in range(0, 2 * ND, kc)]

    def step(b, i):
        r = pl.multiple_of(i * TQ, 16)

        def xa_rows(lo, size):
            return xa_s[pl.ds(r + lo, size), :]

        q = jnp.dot(xa_rows(P, TQ), wqk_s[...], preferred_element_type=F32).astype(BF16)
        hs = {}
        if CARRY:
            gb = [2 * P + v for v in LB]
            for j in range(ND):
                g_s[j, 0:2 * P, :] = g_s[j, TQ:TQ + 2 * P, :]
        else:
            gb = [0] + [2 * P + LB[k + 1] for k in range(NP - 1)] + [TQ + 2 * P]

        def loc_proj():
            if CARRY:
                hs['g'] = jnp.dot(xa_rows(2 * P, TQ), win_ref[:, D:2 * D], preferred_element_type=F32)
            else:
                hs['g'] = jnp.dot(xa_rows(0, TQ + 2 * P), win_ref[:, D:2 * D], preferred_element_type=F32)
            hs['u'] = jnp.dot(xa_rows(P, TQ), win_ref[:, 0:D], preferred_element_type=F32)

        def loc_piece(k):
            dw1 = dw1_ref[...].astype(F32)
            off = 2 * P if CARRY else 0
            g = gate(hs['g'][gb[k] - off:gb[k + 1] - off])
            for j in range(ND):
                g_s[j, gb[k]:gb[k + 1], :] = g[:, j * LANES:(j + 1) * LANES]
            u = _gelu(hs['u'][LB[k]:LB[k + 1]])
            tiles = []
            for j in range(ND):
                acc = None
                for t in range(5):
                    lo = P + LB[k] - 2 + t
                    v = g_s[j, lo:lo + LB[k + 1] - LB[k], :] * dw1[t:t + 1, j * LANES:(j + 1) * LANES]
                    acc = v if acc is None else acc + v
                tiles.append((u[:, j * LANES:(j + 1) * LANES] * acc).astype(BF16))
            loc = jnp.dot(jnp.concatenate(tiles, axis=1), wout_ref[...], preferred_element_type=F32)
            for j in range(ND):
                loc_s[j, LB[k]:LB[k + 1], :] = loc[:, j * LANES:(j + 1) * LANES]

        def schunk(c):
            s = jax.lax.dot_general(q, xa_s[P + c * CK:P + (c + 1) * CK, :], NT, preferred_element_type=F32)
            if (c + 1) * CK > T:
                col = c * CK + jax.lax.broadcasted_iota(jnp.int32, (TQ, CK), 1)
                s = jnp.where(col < T, s, -jnp.inf)
            return s

        def vchunk(lo, size):
            return jnp.concatenate([xa_s[P + lo:P + lo + size, 0:D - LANES], v3_s[lo:lo + size, :]], axis=1)

        def rowmax(s):
            t = s[:, 0:128]
            for j in range(1, s.shape[1] // 128):
                t = jnp.maximum(t, s[:, j * 128:(j + 1) * 128])
            return t

        side = [[] for _ in range(NC + 1)]
        for k in range(NP):
            side[P2AT[k]].append(functools.partial(loc_piece, k))
        side[0].append(loc_proj)
        for k, piece in enumerate(merge(w_s, b, i, i % 2, MB, KC)):
            side[KAT[k]].append(piece)
        mrun = None
        acc = None
        s_next = schunk(0)
        for c in range(NC):
            s = s_next
            if c + 1 < NC:
                s_next = schunk(c + 1)
            mc = jnp.max(rowmax(s), axis=-1, keepdims=True)
            mnew = mc if mrun is None else jnp.maximum(mrun, mc)
            p = jnp.exp2(s - mnew).astype(BF16)
            for task in side[c]:
                task()
            d = jnp.dot(p, vchunk(c * CK, CK), preferred_element_type=F32)
            if mrun is None:
                acc = d
            else:
                acc = acc * jnp.exp2(mrun - mnew) + d
            mrun = mnew
        for task in side[NC]:
            task()
        l = acc[:, D - 1:D]
        on_s[...] = (acc * (1.0 / l)).astype(BF16)
        shift(i != 1)

    def batch(b, carry):
        @pl.when(b == 1)
        def _():
            x1_copy().wait()

        def ln_slab(j, c, wait=True):
            r = pl.multiple_of(j * TL, 16) if wait else j * TL
            if wait:
                for g in range(len(XG) - 2):
                    @pl.when(jnp.logical_and(b == 0, j == XG[g]))
                    def _():
                        x0_copy(g).wait()
            xn = _ln(x_ref[b, pl.ds(r, TL), :].astype(F32))
            xa_s[pl.ds(P + r, TL), :] = xn.astype(BF16)
            v3_s[pl.ds(r, TL), :] = _ones_last(xn[:, D - LANES:]).astype(BF16)
            return c
        jax.lax.fori_loop(0, NL - 1, ln_slab, 0)

        @pl.when(b == 0)
        def _():
            x0_copy(len(XG) - 2).wait()
            in_copy('win').wait()
        ln_slab(NL - 1, 0, False)

        if CARRY:
            g0 = gate(jnp.dot(xa_s[0:2 * P, :], win_ref[:, D:2 * D], preferred_element_type=F32))
            for j in range(ND):
                g_s[j, TQ:TQ + 2 * P, :] = g0[:, j * LANES:(j + 1) * LANES]

        @pl.when(b == 0)
        def _():
            for name in ('dw1', 'dw2', 'wout'):
                in_copy(name).wait()

        def main(i, c):
            n = b * NQ + i

            @pl.when(n == LAG)
            def _():
                in_copy('wm').wait()

            @pl.when(n >= LAG + 2)
            def _():
                out_copy(i % 2, *back(b, i, LAG + 2)).wait()
            publish_prev()
            top_up(i != 1)
            step(b, i)

            @pl.when(n >= LAG)
            def _():
                out_copy(i % 2, *back(b, i, LAG)).start()
            return c
        jax.lax.fori_loop(0, NQ, main, 0)
        return carry
    jax.lax.fori_loop(0, B, batch, 0)

    for k in range(LAG):
        out_copy((NQ + k) % 2, *back(B, k, LAG + 2)).wait()
    publish_prev()
    top_up(True)
    n_s[:, 0:H, :] = w_s[:, TQ:TQ + H, :]
    n_s[:, H + TQ:H + TQ + H, :] = jnp.zeros((2 * ND, H, LANES), F32)
    pieces = [merge(win, B, k, (NQ + k) % 2, TMB, TKC) for k, win in enumerate((w_s, n_s))]
    for ps in pieces:
        for piece in ps:
            piece()
    for k in range(LAG):
        out_copy((NQ + k) % 2, *back(B, k, LAG)).start()
    for k in range(LAG):
        out_copy((NQ + k) % 2, *back(B, k, LAG)).wait()


@jax.jit
def pallas_standalone__conformer_family_e_branchformer__speech_kernel(
    x, w_qkv, w_att_out, w_mlp_in, dw_csgu, w_mlp_out, dw_merge, w_merge):
    B, T, D = x.shape
    TQ = 400
    NQ = T // TQ
    assert NQ % 2 == 0
    CK = CFG['CK']
    TP = -(-T // CK) * CK
    P = 16
    H = 8
    hbm = pl.BlockSpec(memory_space=pl.ANY)
    ins = (x, w_qkv, w_att_out, w_mlp_in, dw_csgu, w_mlp_out, dw_merge, w_merge)

    return pl.pallas_call(
        functools.partial(kernel, B=B, T=T, D=D, TQ=TQ, NQ=NQ, TP=TP, P=P, **CFG),
        in_specs=[hbm] * len(ins),
        out_specs=hbm,
        out_shape=jax.ShapeDtypeStruct((B, T, D), x.dtype),
        scratch_shapes=[pltpu.VMEM(a.shape, a.dtype) for a in ins[:-1]] + [
            pltpu.VMEM((2,) + w_merge.shape, w_merge.dtype),
            pltpu.VMEM((P + TP, D), BF16),
            pltpu.VMEM((TP, LANES), BF16),
            pltpu.VMEM((D, D), BF16),
            pltpu.VMEM((D, D), BF16),
            pltpu.VMEM((2 * D // LANES, TQ + 2 * H, LANES), F32),
            pltpu.VMEM((2 * D // LANES, TQ + 2 * H, LANES), F32),
            pltpu.VMEM((D // LANES, TQ + 2 * P, LANES), F32),
            pltpu.VMEM((2, TQ, D), BF16),
            pltpu.VMEM((TQ, D), BF16),
            pltpu.VMEM((D // LANES, TQ, LANES), F32),
            pltpu.SemaphoreType.DMA((8,)),
            pltpu.SemaphoreType.DMA((T // CFG['TL'] + 1,)),
            pltpu.SemaphoreType.DMA((2,)),
        ],
        compiler_params=pltpu.CompilerParams(
            vmem_limit_bytes=110 * 1024 * 1024),
    )(x, w_qkv, w_att_out, w_mlp_in, dw_csgu, w_mlp_out, dw_merge, w_merge)
```

```python
import functools
import jax
import jax.numpy as jnp
from jax.experimental import pallas as pl
from jax.experimental.pallas import tpu as pltpu

F32 = jnp.float32
BF16 = jnp.bfloat16
LOG2E = 1.4426950408889634
NT = (((1,), (1,)), ((), ()))
LANES = 128
CFG = dict(CK=512, P2AT=[1, 2, 3, 4], MAT=[8], MB=[0, 400], LB=[0, 96, 208, 304, 400], TL=400,
           TMB=[0, 400], CARRY=1, KC=1, TKC=1, KAT=[2, 3, 4, 5, 6, 7, 8, 8], TAILT=1, ZAT=0)


def _ln(x, eps=1e-5):
    m = jnp.mean(x, axis=-1, keepdims=True)
    xc = x - m
    v = jnp.mean(xc * xc, axis=-1, keepdims=True)
    return xc * jnp.exp2(jnp.log(v + eps) * (-0.5 * LOG2E))


def _gelu(x):
    c = 0.7978845608028654
    t = x * x
    z = x * (t * (c * 0.044715) + c)
    h = 0.5 * x
    return h * jnp.tanh(z) + h


def _ones_last(xn):
    lane = jax.lax.broadcasted_iota(jnp.int32, xn.shape, 1)
    return jnp.where(lane == LANES - 1, jnp.ones_like(xn), xn)


def kernel(x_hbm, wqkv_hbm, wo_hbm, win_hbm, dw1_hbm, wout_hbm, dw2_hbm, wm_hbm, o_hbm,
           x_ref, wqkv_ref, wo_ref, win_ref, dw1_ref, wout_ref, dw2_ref, wm_ref,
           xa_s, v3_s, wqk_s, wvo_s, w_s, n_s, g_s, o_s, on_s, loc_s, z_s, isem, xsem, osem,
           *, B, T, D, TQ, NQ, TP, CK, P, TL, P2AT, MAT, MB, LB, TMB, CARRY, KC, TKC, KAT, TAILT, ZAT):
    H = 8
    NC = TP // CK
    NB = B * NQ
    ND = D // LANES
    LAG = 2
    NP = len(LB) - 1
    NM = len(MB) - 1
    NL = T // TL
    TK = T % LANES
    assert TP - T == LANES - TK

    names = ['wqk', 'dw1', 'dw2', 'wv', 'wo', 'win', 'wout', 'wm']
    pairs = dict(
        wqk=(wqkv_hbm.at[:, 0:2 * D], wqkv_ref.at[:, 0:2 * D]),
        wv=(wqkv_hbm.at[:, 2 * D:3 * D], wqkv_ref.at[:, 2 * D:3 * D]),
        win=(win_hbm, win_ref), dw1=(dw1_hbm, dw1_ref), wout=(wout_hbm, wout_ref), wo=(wo_hbm, wo_ref),
        dw2=(dw2_hbm, dw2_ref), wm=(wm_hbm, wm_ref.at[1]))

    def in_copy(name):
        src, dst = pairs[name]
        return pltpu.make_async_copy(src, dst, isem.at[names.index(name)])

    XG = [0, 5, 9, 10]

    def x0_copy(g):
        lo, hi = XG[g] * TL, XG[g + 1] * TL
        return pltpu.make_async_copy(x_hbm.at[0, lo:hi, :], x_ref.at[0, lo:hi, :], xsem.at[g])

    def x1_copy():
        return pltpu.make_async_copy(x_hbm.at[1], x_ref.at[1], xsem.at[NL])

    def back(b, i, k):
        wrap = i < k
        bb = jnp.where(wrap, b - 1, b)
        ii = jnp.where(wrap, i + (NQ - k), i - k)
        first = bb < 0
        return jnp.where(first, 0, bb), pl.multiple_of(jnp.where(first, 0, ii) * TQ, 16)

    def out_copy(slot, bb, rr):
        return pltpu.make_async_copy(o_s.at[slot], o_hbm.at[bb, pl.ds(rr, TQ), :], osem.at[slot])

    for name in names[:5]:
        in_copy(name).start()
    for g in range(len(XG) - 2):
        x0_copy(g).start()
    in_copy('win').start()
    x0_copy(len(XG) - 2).start()
    for name in names[6:]:
        in_copy(name).start()
    x1_copy().start()
    xa_s[0:P, :] = jnp.zeros((P, D), BF16)
    xa_s[P + T:, :] = jnp.zeros((xa_s.shape[0] - P - T, D), BF16)
    v3_s[T:TP, :] = jnp.zeros((TP - T, LANES), BF16)
    w_s[...] = jnp.zeros(w_s.shape, F32)
    n_s[...] = jnp.zeros(n_s.shape, F32)
    on_s[...] = jnp.zeros(on_s.shape, BF16)
    loc_s[...] = jnp.zeros(loc_s.shape, F32)
    wm_ref[0] = jnp.zeros(wm_ref.shape[1:], BF16)
    in_copy('wqk').wait()
    wqk_s[...] = (jax.lax.dot_general(wqkv_ref[:, 0:D], wqkv_ref[:, D:2 * D], NT, preferred_element_type=F32)
                  * (D ** -0.5 * LOG2E)).astype(BF16)
    in_copy('wv').wait()
    in_copy('wo').wait()
    wvo = jnp.dot(wqkv_ref[:, 2 * D:3 * D], wo_ref[...], preferred_element_type=F32)
    wvo_s[...] = (wvo - wvo[D - 1:D, :]).astype(BF16)

    def publish_prev():
        for j in range(ND):
            n_s[ND + j, H:H + TQ, :] = loc_s[j]
        glob = jnp.dot(on_s[...], wvo_s[...], preferred_element_type=F32)
        for j in range(ND):
            n_s[j, H:H + TQ, :] = glob[:, j * LANES:(j + 1) * LANES]

    def edge(rows, keep):
        return jnp.where(keep, rows, jnp.zeros_like(rows))

    def top_up(keep):
        w_s[:, H + TQ:H + TQ + H, :] = edge(n_s[:, H:2 * H, :], keep)

    def shift(keep):
        w_s[:, 0:H, :] = edge(w_s[:, TQ:TQ + H, :], keep)
        w_s[:, H:H + TQ, :] = n_s[:, H:H + TQ, :]

    def gate(h):
        return _ln(_gelu(h))

    def merge(win, b, i, slot, bounds, kc):
        bm, rm = back(b, i, LAG)
        wslot = jnp.logical_or(b > 0, i >= LAG).astype(jnp.int32)
        ys = {}

        def piece(k, j0):
            lo, sz = bounds[k], bounds[k + 1] - bounds[k]
            dw2 = dw2_ref[...].astype(F32)
            dw2 = dw2 + (jax.lax.broadcasted_iota(jnp.int32, dw2.shape, 0) == 2).astype(F32)
            tiles = []
            for j in range(j0, j0 + kc):
                acc = None
                for t in range(5):
                    v = (win[j, lo + H - 2 + t:lo + H - 2 + t + sz, :]
                         * dw2[t:t + 1, j * LANES:(j + 1) * LANES])
                    acc = v if acc is None else acc + v
                tiles.append(acc.astype(BF16))
            d = jnp.dot(jnp.concatenate(tiles, axis=1), wm_ref[wslot, j0 * LANES:(j0 + kc) * LANES, :],
                        preferred_element_type=F32)
            ys[k] = d if j0 == 0 else ys[k] + d
            if j0 + kc == 2 * ND:
                xr = x_ref[bm, pl.ds(rm + lo, sz), :].astype(F32)
                o_s[slot, lo:lo + sz, :] = (xr + ys[k]).astype(o_s.dtype)
        return [functools.partial(piece, k, j0) for k in range(len(bounds) - 1) for j0 in range(0, 2 * ND, kc)]

    def step(b, i):
        r = pl.multiple_of(i * TQ, 16)

        def xa_rows(lo, size):
            return xa_s[pl.ds(r + lo, size), :]

        q = jnp.dot(xa_rows(P, TQ), wqk_s[...], preferred_element_type=F32).astype(BF16)
        hs = {}
        if CARRY:
            gb = [2 * P + v for v in LB]
            for j in range(ND):
                g_s[j, 0:2 * P, :] = g_s[j, TQ:TQ + 2 * P, :]
        else:
            gb = [0] + [2 * P + LB[k + 1] for k in range(NP - 1)] + [TQ + 2 * P]

        def loc_proj():
            if CARRY:
                hs['g'] = jnp.dot(xa_rows(2 * P, TQ), win_ref[:, D:2 * D], preferred_element_type=F32)
            else:
                hs['g'] = jnp.dot(xa_rows(0, TQ + 2 * P), win_ref[:, D:2 * D], preferred_element_type=F32)
            hs['u'] = jnp.dot(xa_rows(P, TQ), win_ref[:, 0:D], preferred_element_type=F32)

        def loc_piece(k):
            dw1 = dw1_ref[...].astype(F32)
            off = 2 * P if CARRY else 0
            g = gate(hs['g'][gb[k] - off:gb[k + 1] - off])
            for j in range(ND):
                g_s[j, gb[k]:gb[k + 1], :] = g[:, j * LANES:(j + 1) * LANES]
            u = _gelu(hs['u'][LB[k]:LB[k + 1]])
            tiles = []
            for j in range(ND):
                acc = None
                for t in range(5):
                    lo = P + LB[k] - 2 + t
                    v = g_s[j, lo:lo + LB[k + 1] - LB[k], :] * dw1[t:t + 1, j * LANES:(j + 1) * LANES]
                    acc = v if acc is None else acc + v
                tiles.append((u[:, j * LANES:(j + 1) * LANES] * acc).astype(BF16))
            loc = jnp.dot(jnp.concatenate(tiles, axis=1), wout_ref[...], preferred_element_type=F32)
            for j in range(ND):
                loc_s[j, LB[k]:LB[k + 1], :] = loc[:, j * LANES:(j + 1) * LANES]

        def tail_scores():
            st = jax.lax.dot_general(z_s[...], xa_rows(P, TQ), NT, preferred_element_type=F32)
            pad = jnp.full((TQ, LANES - TK), -jnp.inf, F32)
            hs['tail'] = jnp.concatenate([st.T, pad], axis=1)

        def schunk(c):
            if TAILT and (c + 1) * CK > T:
                s = jax.lax.dot_general(q, xa_s[P + c * CK:P + T - TK, :], NT, preferred_element_type=F32)
                return jnp.concatenate([s, hs['tail']], axis=1)
            s = jax.lax.dot_general(q, xa_s[P + c * CK:P + (c + 1) * CK, :], NT, preferred_element_type=F32)
            if (c + 1) * CK > T:
                col = c * CK + jax.lax.broadcasted_iota(jnp.int32, (TQ, CK), 1)
                s = jnp.where(col < T, s, -jnp.inf)
            return s

        def vchunk(lo, size):
            return jnp.concatenate([xa_s[P + lo:P + lo + size, 0:D - LANES], v3_s[lo:lo + size, :]], axis=1)

        def rowmax(s):
            t = s[:, 0:128]
            for j in range(1, s.shape[1] // 128):
                t = jnp.maximum(t, s[:, j * 128:(j + 1) * 128])
            return t

        side = [[] for _ in range(NC + 1)]
        for k in range(NP):
            side[P2AT[k]].append(functools.partial(loc_piece, k))
        side[0].append(loc_proj)
        if TAILT:
            side[ZAT].append(tail_scores)
        for k, piece in enumerate(merge(w_s, b, i, i % 2, MB, KC)):
            side[KAT[k]].append(piece)
        mrun = None
        acc = None
        s_next = schunk(0)
        for c in range(NC):
            s = s_next
            if c + 1 < NC:
                s_next = schunk(c + 1)
            mc = jnp.max(rowmax(s), axis=-1, keepdims=True)
            mnew = mc if mrun is None else jnp.maximum(mrun, mc)
            p = jnp.exp2(s - mnew).astype(BF16)
            for task in side[c]:
                task()
            d = jnp.dot(p, vchunk(c * CK, CK), preferred_element_type=F32)
            if mrun is None:
                acc = d
            else:
                acc = acc * jnp.exp2(mrun - mnew) + d
            mrun = mnew
        for task in side[NC]:
            task()
        l = acc[:, D - 1:D]
        on_s[...] = (acc * (1.0 / l)).astype(BF16)
        shift(i != 1)

    def batch(b, carry):
        @pl.when(b == 1)
        def _():
            x1_copy().wait()

        def ln_slab(j, c, wait=True):
            r = pl.multiple_of(j * TL, 16) if wait else j * TL
            if wait:
                for g in range(len(XG) - 2):
                    @pl.when(jnp.logical_and(b == 0, j == XG[g]))
                    def _():
                        x0_copy(g).wait()
            xn = _ln(x_ref[b, pl.ds(r, TL), :].astype(F32))
            xa_s[pl.ds(P + r, TL), :] = xn.astype(BF16)
            v3_s[pl.ds(r, TL), :] = _ones_last(xn[:, D - LANES:]).astype(BF16)
            return c
        jax.lax.fori_loop(0, NL - 1, ln_slab, 0)

        @pl.when(b == 0)
        def _():
            x0_copy(len(XG) - 2).wait()
            in_copy('win').wait()
        ln_slab(NL - 1, 0, False)

        if TAILT:
            z_s[...] = jax.lax.dot_general(xa_s[P + T - TK:P + T, :], wqk_s[...], NT,
                                           preferred_element_type=F32).astype(BF16)
        if CARRY:
            g0 = gate(jnp.dot(xa_s[0:2 * P, :], win_ref[:, D:2 * D], preferred_element_type=F32))
            for j in range(ND):
                g_s[j, TQ:TQ + 2 * P, :] = g0[:, j * LANES:(j + 1) * LANES]

        @pl.when(b == 0)
        def _():
            for name in ('dw1', 'dw2', 'wout'):
                in_copy(name).wait()

        def main(i, c):
            n = b * NQ + i

            @pl.when(n == LAG)
            def _():
                in_copy('wm').wait()

            @pl.when(n >= LAG + 2)
            def _():
                out_copy(i % 2, *back(b, i, LAG + 2)).wait()
            publish_prev()
            top_up(i != 1)
            step(b, i)

            @pl.when(n >= LAG)
            def _():
                out_copy(i % 2, *back(b, i, LAG)).start()
            return c
        jax.lax.fori_loop(0, NQ, main, 0)
        return carry
    jax.lax.fori_loop(0, B, batch, 0)

    for k in range(LAG):
        out_copy((NQ + k) % 2, *back(B, k, LAG + 2)).wait()
    publish_prev()
    top_up(True)
    n_s[:, 0:H, :] = w_s[:, TQ:TQ + H, :]
    n_s[:, H + TQ:H + TQ + H, :] = jnp.zeros((2 * ND, H, LANES), F32)
    pieces = [merge(win, B, k, (NQ + k) % 2, TMB, TKC) for k, win in enumerate((w_s, n_s))]
    for ps in pieces:
        for piece in ps:
            piece()
    for k in range(LAG):
        out_copy((NQ + k) % 2, *back(B, k, LAG)).start()
    for k in range(LAG):
        out_copy((NQ + k) % 2, *back(B, k, LAG)).wait()


@jax.jit
def pallas_standalone__conformer_family_e_branchformer__speech_kernel(
    x, w_qkv, w_att_out, w_mlp_in, dw_csgu, w_mlp_out, dw_merge, w_merge):
    B, T, D = x.shape
    TQ = 400
    NQ = T // TQ
    assert NQ % 2 == 0
    CK = CFG['CK']
    TP = -(-T // CK) * CK
    P = 16
    H = 8
    hbm = pl.BlockSpec(memory_space=pl.ANY)
    ins = (x, w_qkv, w_att_out, w_mlp_in, dw_csgu, w_mlp_out, dw_merge, w_merge)

    return pl.pallas_call(
        functools.partial(kernel, B=B, T=T, D=D, TQ=TQ, NQ=NQ, TP=TP, P=P, **CFG),
        in_specs=[hbm] * len(ins),
        out_specs=hbm,
        out_shape=jax.ShapeDtypeStruct((B, T, D), x.dtype),
        scratch_shapes=[pltpu.VMEM(a.shape, a.dtype) for a in ins[:-1]] + [
            pltpu.VMEM((2,) + w_merge.shape, w_merge.dtype),
            pltpu.VMEM((P + TP, D), BF16),
            pltpu.VMEM((TP, LANES), BF16),
            pltpu.VMEM((D, D), BF16),
            pltpu.VMEM((D, D), BF16),
            pltpu.VMEM((2 * D // LANES, TQ + 2 * H, LANES), F32),
            pltpu.VMEM((2 * D // LANES, TQ + 2 * H, LANES), F32),
            pltpu.VMEM((D // LANES, TQ + 2 * P, LANES), F32),
            pltpu.VMEM((2, TQ, D), BF16),
            pltpu.VMEM((TQ, D), BF16),
            pltpu.VMEM((D // LANES, TQ, LANES), F32),
            pltpu.VMEM((T % LANES, D), BF16),
            pltpu.SemaphoreType.DMA((8,)),
            pltpu.SemaphoreType.DMA((T // CFG['TL'] + 1,)),
            pltpu.SemaphoreType.DMA((2,)),
        ],
        compiler_params=pltpu.CompilerParams(
            vmem_limit_bytes=110 * 1024 * 1024),
    )(x, w_qkv, w_att_out, w_mlp_in, dw_csgu, w_mlp_out, dw_merge, w_merge)
```

```python
import functools
import jax
import jax.numpy as jnp
from jax.experimental import pallas as pl
from jax.experimental.pallas import tpu as pltpu

F32 = jnp.float32
BF16 = jnp.bfloat16
LOG2E = 1.4426950408889634
NT = (((1,), (1,)), ((), ()))
LANES = 128
CFG = dict(CK=512, P2AT=[1, 2, 3, 4], LB=[0, 96, 208, 304, 400], TL=400, KAT=[2, 3, 4, 5, 6, 7, 8, 8],
           ZAT=3)


def _ln(x, eps=1e-5):
    m = jnp.mean(x, axis=-1, keepdims=True)
    xc = x - m
    v = jnp.mean(xc * xc, axis=-1, keepdims=True)
    return xc * jnp.exp2(jnp.log(v + eps) * (-0.5 * LOG2E))


def _gelu(x):
    c = 0.7978845608028654
    t = x * x
    z = x * (t * (c * 0.044715) + c)
    h = 0.5 * x
    return h * jnp.tanh(z) + h


def _ones_last(xn):
    lane = jax.lax.broadcasted_iota(jnp.int32, xn.shape, 1)
    return jnp.where(lane == LANES - 1, jnp.ones_like(xn), xn)


def kernel(x_hbm, wqkv_hbm, wo_hbm, win_hbm, dw1_hbm, wout_hbm, dw2_hbm, wm_hbm, o_hbm,
           x_ref, wqkv_ref, wo_ref, win_ref, dw1_ref, wout_ref, dw2_ref, wm_ref,
           xa_s, v3_s, wqk_s, wvo_s, w_s, g_s, o_s, oe_s, on_s, loc_s, z_s, isem, xsem, osem,
           *, B, T, D, TQ, NQ, TP, CK, P, TL, P2AT, LB, KAT, ZAT):
    NC = TP // CK
    ND = D // LANES
    NP = len(LB) - 1
    NL = T // TL
    TK = T % LANES
    assert TP - T == LANES - TK
    SK = 16
    HW = SK + 8
    XG = [0, 5, 9, 10]

    names = ['wqk', 'dw1', 'dw2', 'wv', 'wo', 'win', 'wout', 'wm']
    pairs = dict(
        wqk=(wqkv_hbm.at[:, 0:2 * D], wqkv_ref.at[:, 0:2 * D]),
        wv=(wqkv_hbm.at[:, 2 * D:3 * D], wqkv_ref.at[:, 2 * D:3 * D]),
        win=(win_hbm, win_ref), dw1=(dw1_hbm, dw1_ref), wout=(wout_hbm, wout_ref), wo=(wo_hbm, wo_ref),
        dw2=(dw2_hbm, dw2_ref), wm=(wm_hbm, wm_ref.at[1]))

    def in_copy(name):
        src, dst = pairs[name]
        return pltpu.make_async_copy(src, dst, isem.at[names.index(name)])

    def x0_copy(g):
        lo, hi = XG[g] * TL, XG[g + 1] * TL
        return pltpu.make_async_copy(x_hbm.at[0, lo:hi, :], x_ref.at[0, SK + lo:SK + hi, :], xsem.at[g])

    def x1_copy():
        return pltpu.make_async_copy(x_hbm.at[1], x_ref.at[1, SK:SK + T, :], xsem.at[len(XG) - 1])

    def back(b, i, k):
        wrap = i < k
        bb = jnp.where(wrap, b - 1, b)
        ii = jnp.where(wrap, i + (NQ - k), i - k)
        first = bb < 0
        return jnp.where(first, 0, bb), jnp.where(first, 0, ii)

    def out_ops(op, slot, bb, ii):
        @pl.when(ii > 0)
        def _():
            r = pl.multiple_of(ii * TQ - SK, 16)
            op(pltpu.make_async_copy(o_s.at[slot], o_hbm.at[bb, pl.ds(r, TQ), :], osem.at[slot]))

        @pl.when(ii == 0)
        def _():
            op(pltpu.make_async_copy(o_s.at[slot, SK:TQ, :], o_hbm.at[bb, 0:TQ - SK, :], osem.at[slot]))

    def end_copy(bb):
        return pltpu.make_async_copy(oe_s, o_hbm.at[bb, T - SK:T, :], osem.at[2])

    start = lambda cp: cp.start()
    wait = lambda cp: cp.wait()

    for name in names[:5]:
        in_copy(name).start()
    for g in range(len(XG) - 2):
        x0_copy(g).start()
    in_copy('win').start()
    x0_copy(len(XG) - 2).start()
    for name in names[6:]:
        in_copy(name).start()
    x1_copy().start()
    xa_s[0:P, :] = jnp.zeros((P, D), BF16)
    xa_s[P + T:, :] = jnp.zeros((xa_s.shape[0] - P - T, D), BF16)
    v3_s[T:TP, :] = jnp.zeros((TP - T, LANES), BF16)
    for b in range(B):
        x_ref[b, 0:SK, :] = jnp.zeros((SK, D), BF16)
    w_s[...] = jnp.zeros(w_s.shape, F32)
    on_s[...] = jnp.zeros(on_s.shape, BF16)
    loc_s[...] = jnp.zeros(loc_s.shape, F32)
    wm_ref[0] = jnp.zeros(wm_ref.shape[1:], BF16)
    in_copy('wqk').wait()
    wqk_s[...] = (jax.lax.dot_general(wqkv_ref[:, 0:D], wqkv_ref[:, D:2 * D], NT, preferred_element_type=F32)
                  * (D ** -0.5 * LOG2E)).astype(BF16)
    in_copy('wv').wait()
    in_copy('wo').wait()
    wvo = jnp.dot(wqkv_ref[:, 2 * D:3 * D], wo_ref[...], preferred_element_type=F32)
    wvo_s[...] = (wvo - wvo[D - 1:D, :]).astype(BF16)

    def publish_prev(keep):
        tail = w_s[:, TQ:TQ + HW, :]
        w_s[:, 0:HW, :] = jnp.where(keep, tail, jnp.zeros_like(tail))
        for j in range(ND):
            w_s[ND + j, HW:HW + TQ, :] = loc_s[j]
        glob = jnp.dot(on_s[...], wvo_s[...], preferred_element_type=F32)
        for j in range(ND):
            w_s[j, HW:HW + TQ, :] = glob[:, j * LANES:(j + 1) * LANES]

    def gate(h):
        return _ln(_gelu(h))

    def merge(bm, im, wslot, lo, sz, dst):
        ys = {}

        def piece(j):
            dw2 = dw2_ref[...].astype(F32)
            dw2 = dw2 + (jax.lax.broadcasted_iota(jnp.int32, dw2.shape, 0) == 2).astype(F32)
            acc = None
            for t in range(5):
                o = HW - SK + lo - 2 + t
                v = w_s[j, o:o + sz, :] * dw2[t:t + 1, j * LANES:(j + 1) * LANES]
                acc = v if acc is None else acc + v
            d = jnp.dot(acc.astype(BF16), wm_ref[wslot, j * LANES:(j + 1) * LANES, :], preferred_element_type=F32)
            ys['y'] = d if j == 0 else ys['y'] + d
            if j == 2 * ND - 1:
                xr = x_ref[bm, pl.ds(pl.multiple_of(im * TQ + lo, 16), sz), :].astype(F32)
                dst[...] = (xr + ys['y']).astype(BF16)
        return [functools.partial(piece, j) for j in range(2 * ND)]

    def sequence_end(bm):
        for task in merge(bm, NQ - 1, 1, TQ, SK, oe_s):
            task()
        end_copy(bm).start()

    def step(b, i):
        r = pl.multiple_of(i * TQ, 16)

        def xa_rows(lo, size):
            return xa_s[pl.ds(r + lo, size), :]

        q = jnp.dot(xa_rows(P, TQ), wqk_s[...], preferred_element_type=F32).astype(BF16)
        hs = {}
        gb = [2 * P + v for v in LB]
        for j in range(ND):
            g_s[j, 0:2 * P, :] = g_s[j, TQ:TQ + 2 * P, :]

        def loc_proj():
            hs['g'] = jnp.dot(xa_rows(2 * P, TQ), win_ref[:, D:2 * D], preferred_element_type=F32)
            hs['u'] = jnp.dot(xa_rows(P, TQ), win_ref[:, 0:D], preferred_element_type=F32)

        def loc_piece(k):
            dw1 = dw1_ref[...].astype(F32)
            g = gate(hs['g'][LB[k]:LB[k + 1]])
            for j in range(ND):
                g_s[j, gb[k]:gb[k + 1], :] = g[:, j * LANES:(j + 1) * LANES]
            u = _gelu(hs['u'][LB[k]:LB[k + 1]])
            tiles = []
            for j in range(ND):
                acc = None
                for t in range(5):
                    lo = P + LB[k] - 2 + t
                    v = g_s[j, lo:lo + LB[k + 1] - LB[k], :] * dw1[t:t + 1, j * LANES:(j + 1) * LANES]
                    acc = v if acc is None else acc + v
                tiles.append((u[:, j * LANES:(j + 1) * LANES] * acc).astype(BF16))
            loc = jnp.dot(jnp.concatenate(tiles, axis=1), wout_ref[...], preferred_element_type=F32)
            for j in range(ND):
                loc_s[j, LB[k]:LB[k + 1], :] = loc[:, j * LANES:(j + 1) * LANES]

        def tail_scores():
            st = jax.lax.dot_general(z_s[...], xa_rows(P, TQ), NT, preferred_element_type=F32)
            pad = jnp.full((TQ, LANES - TK), -jnp.inf, F32)
            hs['tail'] = jnp.concatenate([st.T, pad], axis=1)

        def schunk(c):
            if (c + 1) * CK > T:
                s = jax.lax.dot_general(q, xa_s[P + c * CK:P + T - TK, :], NT, preferred_element_type=F32)
                return jnp.concatenate([s, hs['tail']], axis=1)
            return jax.lax.dot_general(q, xa_s[P + c * CK:P + (c + 1) * CK, :], NT, preferred_element_type=F32)

        def vchunk(lo, size):
            return jnp.concatenate([xa_s[P + lo:P + lo + size, 0:D - LANES], v3_s[lo:lo + size, :]], axis=1)

        def rowmax(s):
            t = s[:, 0:128]
            for j in range(1, s.shape[1] // 128):
                t = jnp.maximum(t, s[:, j * 128:(j + 1) * 128])
            return t

        side = [[] for _ in range(NC + 1)]
        for k in range(NP):
            side[P2AT[k]].append(functools.partial(loc_piece, k))
        side[0].append(loc_proj)
        side[ZAT].append(tail_scores)
        bm, im = back(b, i, 1)
        wslot = jnp.logical_or(b > 0, i > 0).astype(jnp.int32)
        for k, piece in enumerate(merge(bm, im, wslot, 0, TQ, o_s.at[i % 2])):
            side[KAT[k]].append(piece)
        mrun = None
        acc = None
        s_next = schunk(0)
        for c in range(NC):
            s = s_next
            if c + 1 < NC:
                s_next = schunk(c + 1)
            mc = jnp.max(rowmax(s), axis=-1, keepdims=True)
            mnew = mc if mrun is None else jnp.maximum(mrun, mc)
            p = jnp.exp2(s - mnew).astype(BF16)
            for task in side[c]:
                task()
            d = jnp.dot(p, vchunk(c * CK, CK), preferred_element_type=F32)
            if mrun is None:
                acc = d
            else:
                acc = acc * jnp.exp2(mrun - mnew) + d
            mrun = mnew
        for task in side[NC]:
            task()
        l = acc[:, D - 1:D]
        on_s[...] = (acc * (1.0 / l)).astype(BF16)

    def batch(b, carry):
        @pl.when(b == 1)
        def _():
            x1_copy().wait()

        def ln_slab(j, c, wait=True):
            r = pl.multiple_of(j * TL, 16) if wait else j * TL
            if wait:
                for g in range(len(XG) - 2):
                    @pl.when(jnp.logical_and(b == 0, j == XG[g]))
                    def _():
                        x0_copy(g).wait()
            xn = _ln(x_ref[b, pl.ds(SK + r, TL), :].astype(F32))
            xa_s[pl.ds(P + r, TL), :] = xn.astype(BF16)
            v3_s[pl.ds(r, TL), :] = _ones_last(xn[:, D - LANES:]).astype(BF16)
            return c
        jax.lax.fori_loop(0, NL - 1, ln_slab, 0)

        @pl.when(b == 0)
        def _():
            x0_copy(len(XG) - 2).wait()
            in_copy('win').wait()
        ln_slab(NL - 1, 0, False)
        z_s[...] = jax.lax.dot_general(xa_s[P + T - TK:P + T, :], wqk_s[...], NT,
                                       preferred_element_type=F32).astype(BF16)
        g0 = gate(jnp.dot(xa_s[0:2 * P, :], win_ref[:, D:2 * D], preferred_element_type=F32))
        for j in range(ND):
            g_s[j, TQ:TQ + 2 * P, :] = g0[:, j * LANES:(j + 1) * LANES]

        @pl.when(b == 0)
        def _():
            for name in ('dw1', 'dw2', 'wout'):
                in_copy(name).wait()

        def main(i, c):
            n = b * NQ + i

            @pl.when(n == 1)
            def _():
                in_copy('wm').wait()

            @pl.when(n >= 3)
            def _():
                out_ops(wait, i % 2, *back(b, i, 3))
            publish_prev(i != 1)
            step(b, i)

            @pl.when(n >= 1)
            def _():
                out_ops(start, i % 2, *back(b, i, 1))

            @pl.when(jnp.logical_and(b > 0, i == 0))
            def _():
                sequence_end(b - 1)
            return c
        jax.lax.fori_loop(0, NQ, main, 0)
        return carry
    jax.lax.fori_loop(0, B, batch, 0)

    out_ops(wait, 0, *back(B, 0, 3))
    for b in range(B - 1):
        end_copy(b).wait()
    publish_prev(True)
    for task in merge(B - 1, NQ - 1, 1, 0, TQ, o_s.at[0]):
        task()
    out_ops(start, 0, B - 1, NQ - 1)
    sequence_end(B - 1)
    out_ops(wait, 1, *back(B, 0, 2))
    out_ops(wait, 0, B - 1, NQ - 1)
    end_copy(B - 1).wait()


@jax.jit
def pallas_standalone__conformer_family_e_branchformer__speech_kernel(
    x, w_qkv, w_att_out, w_mlp_in, dw_csgu, w_mlp_out, dw_merge, w_merge):
    B, T, D = x.shape
    TQ = 400
    NQ = T // TQ
    assert B == 2 and NQ % 2 == 0
    CK = CFG['CK']
    TP = -(-T // CK) * CK
    P = 16
    hbm = pl.BlockSpec(memory_space=pl.ANY)
    ins = (x, w_qkv, w_att_out, w_mlp_in, dw_csgu, w_mlp_out, dw_merge, w_merge)

    return pl.pallas_call(
        functools.partial(kernel, B=B, T=T, D=D, TQ=TQ, NQ=NQ, TP=TP, P=P, **CFG),
        in_specs=[hbm] * len(ins),
        out_specs=hbm,
        out_shape=jax.ShapeDtypeStruct((B, T, D), x.dtype),
        scratch_shapes=[pltpu.VMEM((B, 16 + T, D), x.dtype)] + [pltpu.VMEM(a.shape, a.dtype) for a in ins[1:-1]] + [
            pltpu.VMEM((2,) + w_merge.shape, w_merge.dtype),
            pltpu.VMEM((P + TP, D), BF16),
            pltpu.VMEM((TP, LANES), BF16),
            pltpu.VMEM((D, D), BF16),
            pltpu.VMEM((D, D), BF16),
            pltpu.VMEM((2 * D // LANES, TQ + 32, LANES), F32),
            pltpu.VMEM((D // LANES, TQ + 2 * P, LANES), F32),
            pltpu.VMEM((2, TQ, D), BF16),
            pltpu.VMEM((16, D), BF16),
            pltpu.VMEM((TQ, D), BF16),
            pltpu.VMEM((D // LANES, TQ, LANES), F32),
            pltpu.VMEM((T % LANES, D), BF16),
            pltpu.SemaphoreType.DMA((8,)),
            pltpu.SemaphoreType.DMA((4,)),
            pltpu.SemaphoreType.DMA((3,)),
        ],
        compiler_params=pltpu.CompilerParams(
            vmem_limit_bytes=110 * 1024 * 1024),
    )(x, w_qkv, w_att_out, w_mlp_in, dw_csgu, w_mlp_out, dw_merge, w_merge)
```

```python
import functools
import jax
import jax.numpy as jnp
from jax.experimental import pallas as pl
from jax.experimental.pallas import tpu as pltpu

F32 = jnp.float32
BF16 = jnp.bfloat16
LOG2E = 1.4426950408889634
NT = (((1,), (1,)), ((), ()))
LANES = 128
CFG = dict(CK=512, P2AT=[1, 2, 3, 4], LB=[0, 96, 208, 304, 400], TL=400, KAT=[2, 3, 4, 5, 6, 7, 8, 8],
           ZAT=0, TS=448, LNAT=0)


def _ln(x, eps=1e-5):
    m = jnp.mean(x, axis=-1, keepdims=True)
    xc = x - m
    v = jnp.mean(xc * xc, axis=-1, keepdims=True)
    return xc * jnp.exp2(jnp.log(v + eps) * (-0.5 * LOG2E))


def _gelu(x):
    c = 0.7978845608028654
    t = x * x
    z = x * (t * (c * 0.044715) + c)
    h = 0.5 * x
    return h * jnp.tanh(z) + h


def _ones_last(xn):
    lane = jax.lax.broadcasted_iota(jnp.int32, xn.shape, 1)
    return jnp.where(lane == LANES - 1, jnp.ones_like(xn), xn)


def kernel(x_hbm, wqkv_hbm, wo_hbm, win_hbm, dw1_hbm, wout_hbm, dw2_hbm, wm_hbm, o_hbm,
           x_ref, wqkv_ref, wo_ref, win_ref, dw1_ref, wout_ref, dw2_ref, wm_ref,
           xa_s, v3_s, xb_s, vb_s, wqk_s, wvo_s, w_s, g_s, o_s, oe_s, on_s, loc_s, z_s, isem, xsem, osem,
           *, B, T, D, TQ, NQ, TP, CK, P, TL, P2AT, LB, KAT, ZAT, TS, LNAT):
    NC = TP // CK
    ND = D // LANES
    NP = len(LB) - 1
    NL = T // TL
    TK = T % LANES
    assert TP - T == LANES - TK
    SK = 16
    HW = SK + 8
    XG = [0, 5, 9, 10]

    names = ['wqk', 'dw1', 'dw2', 'wv', 'wo', 'win', 'wout', 'wm']
    pairs = dict(
        wqk=(wqkv_hbm.at[:, 0:2 * D], wqkv_ref.at[:, 0:2 * D]),
        wv=(wqkv_hbm.at[:, 2 * D:3 * D], wqkv_ref.at[:, 2 * D:3 * D]),
        win=(win_hbm, win_ref), dw1=(dw1_hbm, dw1_ref), wout=(wout_hbm, wout_ref), wo=(wo_hbm, wo_ref),
        dw2=(dw2_hbm, dw2_ref), wm=(wm_hbm, wm_ref.at[1]))

    def in_copy(name):
        src, dst = pairs[name]
        return pltpu.make_async_copy(src, dst, isem.at[names.index(name)])

    def x0_copy(g):
        lo, hi = XG[g] * TL, XG[g + 1] * TL
        return pltpu.make_async_copy(x_hbm.at[0, lo:hi, :], x_ref.at[0, SK + lo:SK + hi, :], xsem.at[g])

    def x1_copy():
        return pltpu.make_async_copy(x_hbm.at[1], x_ref.at[1, SK:SK + T, :], xsem.at[len(XG) - 1])

    def back(b, i, k):
        wrap = i < k
        bb = jnp.where(wrap, b - 1, b)
        ii = jnp.where(wrap, i + (NQ - k), i - k)
        first = bb < 0
        return jnp.where(first, 0, bb), jnp.where(first, 0, ii)

    def out_start(slot, bb, ii):
        r = pl.multiple_of(ii * TQ, 16)
        rh = pl.multiple_of(jnp.where(ii > 0, r - SK, T - SK), 16)
        pltpu.make_async_copy(o_s.at[slot, 0:SK, :], o_hbm.at[bb, pl.ds(rh, SK), :], osem.at[slot]).start()
        pltpu.make_async_copy(o_s.at[slot, SK:TQ, :], o_hbm.at[bb, pl.ds(r, TQ - SK), :], osem.at[slot]).start()

    def out_wait(slot):
        pltpu.make_async_copy(o_s.at[slot], o_s.at[slot], osem.at[slot]).wait()

    def end_copy(bb):
        return pltpu.make_async_copy(oe_s, o_hbm.at[bb, T - SK:T, :], osem.at[2])

    for name in names[:5]:
        in_copy(name).start()
    for g in range(len(XG) - 2):
        x0_copy(g).start()
    in_copy('win').start()
    x0_copy(len(XG) - 2).start()
    for name in names[6:]:
        in_copy(name).start()
    x1_copy().start()
    xa_s[0:P, :] = jnp.zeros((P, D), BF16)
    xa_s[P + T:, :] = jnp.zeros((xa_s.shape[0] - P - T, D), BF16)
    v3_s[T:TP, :] = jnp.zeros((TP - T, LANES), BF16)
    for b in range(B):
        x_ref[b, 0:SK, :] = jnp.zeros((SK, D), BF16)
    w_s[...] = jnp.zeros(w_s.shape, F32)
    on_s[...] = jnp.zeros(on_s.shape, BF16)
    loc_s[...] = jnp.zeros(loc_s.shape, F32)
    wm_ref[0] = jnp.zeros(wm_ref.shape[1:], BF16)
    in_copy('wqk').wait()
    wqk_s[...] = (jax.lax.dot_general(wqkv_ref[:, 0:D], wqkv_ref[:, D:2 * D], NT, preferred_element_type=F32)
                  * (D ** -0.5 * LOG2E)).astype(BF16)
    in_copy('wv').wait()
    in_copy('wo').wait()
    wvo = jnp.dot(wqkv_ref[:, 2 * D:3 * D], wo_ref[...], preferred_element_type=F32)
    wvo_s[...] = (wvo - wvo[D - 1:D, :]).astype(BF16)

    def publish_prev(keep):
        tail = w_s[:, TQ:TQ + HW, :]
        w_s[:, 0:HW, :] = jnp.where(keep, tail, jnp.zeros_like(tail))
        for j in range(ND):
            w_s[ND + j, HW:HW + TQ, :] = loc_s[j]
        glob = jnp.dot(on_s[...], wvo_s[...], preferred_element_type=F32)
        for j in range(ND):
            w_s[j, HW:HW + TQ, :] = glob[:, j * LANES:(j + 1) * LANES]

    def gate(h):
        return _ln(_gelu(h))

    def merge(bm, im, wslot, lo, sz, dst):
        ys = {}

        def piece(j):
            dw2 = dw2_ref[...].astype(F32)
            dw2 = dw2 + (jax.lax.broadcasted_iota(jnp.int32, dw2.shape, 0) == 2).astype(F32)
            acc = None
            for t in range(5):
                o = HW - SK + lo - 2 + t
                v = w_s[j, o:o + sz, :] * dw2[t:t + 1, j * LANES:(j + 1) * LANES]
                acc = v if acc is None else acc + v
            d = jnp.dot(acc.astype(BF16), wm_ref[wslot, j * LANES:(j + 1) * LANES, :], preferred_element_type=F32)
            ys['y'] = d if j == 0 else ys['y'] + d
            if j == 2 * ND - 1:
                xr = x_ref[bm, pl.ds(pl.multiple_of(im * TQ + lo, 16), sz), :].astype(F32)
                dst[...] = (xr + ys['y']).astype(BF16)
        return [functools.partial(piece, j) for j in range(2 * ND)]

    def sequence_end(bm):
        for task in merge(bm, NQ - 1, 1, TQ, SK, oe_s):
            task()
        end_copy(bm).start()

    def step(b, i):
        r = pl.multiple_of(i * TQ, 16)

        def xa_rows(lo, size):
            return xa_s[pl.ds(r + lo, size), :]

        def ln_lead():
            rl = pl.multiple_of(jnp.clip((i - 1) * TS, 0, T - TS), 16)
            src = jnp.where(jnp.logical_and(b == 0, i == 0), 0, 1)
            xn = _ln(x_ref[src, pl.ds(SK + rl, TS), :].astype(F32))
            xb_s[pl.ds(rl, TS), :] = xn.astype(BF16)
            vb_s[pl.ds(rl, TS), :] = _ones_last(xn[:, D - LANES:]).astype(BF16)

        q = jnp.dot(xa_rows(P, TQ), wqk_s[...], preferred_element_type=F32).astype(BF16)
        hs = {}
        gb = [2 * P + v for v in LB]
        for j in range(ND):
            g_s[j, 0:2 * P, :] = g_s[j, TQ:TQ + 2 * P, :]

        def loc_proj():
            hs['g'] = jnp.dot(xa_rows(2 * P, TQ), win_ref[:, D:2 * D], preferred_element_type=F32)
            hs['u'] = jnp.dot(xa_rows(P, TQ), win_ref[:, 0:D], preferred_element_type=F32)

        def loc_piece(k):
            dw1 = dw1_ref[...].astype(F32)
            g = gate(hs['g'][LB[k]:LB[k + 1]])
            for j in range(ND):
                g_s[j, gb[k]:gb[k + 1], :] = g[:, j * LANES:(j + 1) * LANES]
            u = _gelu(hs['u'][LB[k]:LB[k + 1]])
            tiles = []
            for j in range(ND):
                acc = None
                for t in range(5):
                    lo = P + LB[k] - 2 + t
                    v = g_s[j, lo:lo + LB[k + 1] - LB[k], :] * dw1[t:t + 1, j * LANES:(j + 1) * LANES]
                    acc = v if acc is None else acc + v
                tiles.append((u[:, j * LANES:(j + 1) * LANES] * acc).astype(BF16))
            loc = jnp.dot(jnp.concatenate(tiles, axis=1), wout_ref[...], preferred_element_type=F32)
            for j in range(ND):
                loc_s[j, LB[k]:LB[k + 1], :] = loc[:, j * LANES:(j + 1) * LANES]

        def tail_scores():
            st = jax.lax.dot_general(z_s[...], xa_rows(P, TQ), NT, preferred_element_type=F32)
            pad = jnp.full((TQ, LANES - TK), -jnp.inf, F32)
            hs['tail'] = jnp.concatenate([st.T, pad], axis=1)

        def schunk(c):
            if (c + 1) * CK > T:
                s = jax.lax.dot_general(q, xa_s[P + c * CK:P + T - TK, :], NT, preferred_element_type=F32)
                return jnp.concatenate([s, hs['tail']], axis=1)
            return jax.lax.dot_general(q, xa_s[P + c * CK:P + (c + 1) * CK, :], NT, preferred_element_type=F32)

        def vchunk(lo, size):
            return jnp.concatenate([xa_s[P + lo:P + lo + size, 0:D - LANES], v3_s[lo:lo + size, :]], axis=1)

        def rowmax(s):
            t = s[:, 0:128]
            for j in range(1, s.shape[1] // 128):
                t = jnp.maximum(t, s[:, j * 128:(j + 1) * 128])
            return t

        side = [[] for _ in range(NC + 1)]
        for k in range(NP):
            side[P2AT[k]].append(functools.partial(loc_piece, k))
        side[0].append(loc_proj)
        side[ZAT].append(tail_scores)
        bm, im = back(b, i, 1)
        wslot = jnp.logical_or(b > 0, i > 0).astype(jnp.int32)
        for k, piece in enumerate(merge(bm, im, wslot, 0, TQ, o_s.at[i & 1])):
            side[KAT[k]].append(piece)
        side[LNAT].append(ln_lead)
        mrun = None
        acc = None
        s_next = schunk(0)
        for c in range(NC):
            s = s_next
            if c + 1 < NC:
                s_next = schunk(c + 1)
            mc = jnp.max(rowmax(s), axis=-1, keepdims=True)
            mnew = mc if mrun is None else jnp.maximum(mrun, mc)
            p = jnp.exp2(s - mnew).astype(BF16)
            for task in side[c]:
                task()
            d = jnp.dot(p, vchunk(c * CK, CK), preferred_element_type=F32)
            if mrun is None:
                acc = d
            else:
                acc = acc * jnp.exp2(mrun - mnew) + d
            mrun = mnew
        for task in side[NC]:
            task()
        l = acc[:, D - 1:D]
        on_s[...] = (acc * (1.0 / l)).astype(BF16)

    def ln_slab(j, wait=True):
        r = pl.multiple_of(j * TL, 16) if wait else j * TL
        if wait:
            for g in range(len(XG) - 2):
                @pl.when(j == XG[g])
                def _():
                    x0_copy(g).wait()
        xn = _ln(x_ref[0, pl.ds(SK + r, TL), :].astype(F32))
        xa_s[pl.ds(P + r, TL), :] = xn.astype(BF16)
        v3_s[pl.ds(r, TL), :] = _ones_last(xn[:, D - LANES:]).astype(BF16)

    def sequence_start():
        z_s[...] = jax.lax.dot_general(xa_s[P + T - TK:P + T, :], wqk_s[...], NT,
                                       preferred_element_type=F32).astype(BF16)
        g0 = gate(jnp.dot(xa_s[0:2 * P, :], win_ref[:, D:2 * D], preferred_element_type=F32))
        for j in range(ND):
            g_s[j, TQ:TQ + 2 * P, :] = g0[:, j * LANES:(j + 1) * LANES]

    def cp_slab(j, static=False):
        r = j * TL if static else pl.multiple_of(j * TL, 16)
        xa_s[pl.ds(P + r, TL), :] = xb_s[pl.ds(r, TL), :]
        v3_s[pl.ds(r, TL), :] = vb_s[pl.ds(r, TL), :]

    def batch(b, carry):
        @pl.when(b == 0)
        def _():
            jax.lax.fori_loop(0, NL - 1, lambda j, c: ln_slab(j), None)
            x0_copy(len(XG) - 2).wait()
            in_copy('win').wait()
            ln_slab(NL - 1, False)
            sequence_start()

        @pl.when(b > 0)
        def _():
            jax.lax.fori_loop(1, NL - 2, lambda j, c: cp_slab(j), None)
            cp_slab(0, True)
            cp_slab(NL - 1, True)
            sequence_start()
            cp_slab(NL - 2, True)

        @pl.when(b == 0)
        def _():
            for name in ('dw1', 'dw2', 'wout'):
                in_copy(name).wait()

        def main(i, c):
            n = b * NQ + i

            @pl.when(n == 1)
            def _():
                in_copy('wm').wait()
                x1_copy().wait()

            @pl.when(n >= 3)
            def _():
                out_wait(i & 1)
            publish_prev(i != 1)
            step(b, i)

            @pl.when(n >= 1)
            def _():
                out_start(i & 1, *back(b, i, 1))

            @pl.when(jnp.logical_and(b > 0, i == 0))
            def _():
                sequence_end(b - 1)
            return c
        jax.lax.fori_loop(0, NQ, main, 0)
        return carry
    jax.lax.fori_loop(0, B, batch, 0)

    out_wait(0)
    for b in range(B - 1):
        end_copy(b).wait()
    publish_prev(True)
    for task in merge(B - 1, NQ - 1, 1, 0, TQ, o_s.at[0]):
        task()
    out_start(0, B - 1, NQ - 1)
    sequence_end(B - 1)
    out_wait(1)
    out_wait(0)
    end_copy(B - 1).wait()


@jax.jit
def pallas_standalone__conformer_family_e_branchformer__speech_kernel(
    x, w_qkv, w_att_out, w_mlp_in, dw_csgu, w_mlp_out, dw_merge, w_merge):
    B, T, D = x.shape
    TQ = 400
    NQ = T // TQ
    assert B == 2 and NQ % 2 == 0
    CK = CFG['CK']
    TP = -(-T // CK) * CK
    P = 16
    hbm = pl.BlockSpec(memory_space=pl.ANY)
    ins = (x, w_qkv, w_att_out, w_mlp_in, dw_csgu, w_mlp_out, dw_merge, w_merge)

    return pl.pallas_call(
        functools.partial(kernel, B=B, T=T, D=D, TQ=TQ, NQ=NQ, TP=TP, P=P, **CFG),
        in_specs=[hbm] * len(ins),
        out_specs=hbm,
        out_shape=jax.ShapeDtypeStruct((B, T, D), x.dtype),
        scratch_shapes=[pltpu.VMEM((B, 16 + T, D), x.dtype)] + [pltpu.VMEM(a.shape, a.dtype) for a in ins[1:-1]] + [
            pltpu.VMEM((2,) + w_merge.shape, w_merge.dtype),
            pltpu.VMEM((P + TP, D), BF16),
            pltpu.VMEM((TP, LANES), BF16),
            pltpu.VMEM((T, D), BF16),
            pltpu.VMEM((T, LANES), BF16),
            pltpu.VMEM((D, D), BF16),
            pltpu.VMEM((D, D), BF16),
            pltpu.VMEM((2 * D // LANES, TQ + 32, LANES), F32),
            pltpu.VMEM((D // LANES, TQ + 2 * P, LANES), F32),
            pltpu.VMEM((2, TQ, D), BF16),
            pltpu.VMEM((16, D), BF16),
            pltpu.VMEM((TQ, D), BF16),
            pltpu.VMEM((D // LANES, TQ, LANES), F32),
            pltpu.VMEM((T % LANES, D), BF16),
            pltpu.SemaphoreType.DMA((8,)),
            pltpu.SemaphoreType.DMA((4,)),
            pltpu.SemaphoreType.DMA((3,)),
        ],
        compiler_params=pltpu.CompilerParams(
            vmem_limit_bytes=110 * 1024 * 1024, disable_bounds_checks=True),
    )(x, w_qkv, w_att_out, w_mlp_in, dw_csgu, w_mlp_out, dw_merge, w_merge)
```

```python
import functools
import jax
import jax.numpy as jnp
from jax.experimental import pallas as pl
from jax.experimental.pallas import tpu as pltpu

F32 = jnp.float32
BF16 = jnp.bfloat16
LOG2E = 1.4426950408889634
NT = (((1,), (1,)), ((), ()))
LANES = 128
CK = 512
LOC_ROWS = (0, 96, 208, 304, 400)
LOC_SLOT = (1, 2, 3, 4)
MERGE_SLOT = (2, 3, 4, 5, 6, 7, 8, 8)
TL = 400
TS = 448
TH = 304


def _ln(x, eps=1e-5):
    m = jnp.mean(x, axis=-1, keepdims=True)
    xc = x - m
    v = jnp.mean(xc * xc, axis=-1, keepdims=True)
    return xc * jnp.exp2(jnp.log(v + eps) * (-0.5 * LOG2E))


def _gelu(x):
    c = 0.7978845608028654
    t = x * x
    z = x * (t * (c * 0.044715) + c)
    h = 0.5 * x
    return h * jnp.tanh(z) + h


def _ones_last(xn):
    lane = jax.lax.broadcasted_iota(jnp.int32, xn.shape, 1)
    return jnp.where(lane == LANES - 1, jnp.ones_like(xn), xn)


def _rowmax(s):
    t = s[:, 0:LANES]
    for j in range(1, s.shape[1] // LANES):
        t = jnp.maximum(t, s[:, j * LANES:(j + 1) * LANES])
    return t


def kernel(x_hbm, wqkv_hbm, wo_hbm, win_hbm, dw1_hbm, wout_hbm, dw2_hbm, wm_hbm, o_hbm,
           x_ref, wqkv_ref, wo_ref, win_ref, dw1_ref, wout_ref, dw2_ref, wm_ref,
           xa_s, v3_s, xb_s, vb_s, wqk_s, wvo_s, w_s, g_s, o_s, oe_s, on_s, loc_s, z_s,
           q_s, s_s, acc_s, m_s, isem, xsem, osem,
           *, B, T, D, TQ, NQ, TP, P):
    NC = TP // CK
    ND = D // LANES
    LB = LOC_ROWS
    NP = len(LB) - 1
    NL = T // TL
    TK = T % LANES
    assert TP - T == LANES - TK
    SK = 16
    HW = SK + 8

    names = ['wqk', 'wv', 'wo', 'win', 'dw1', 'dw2', 'wout', 'wm']
    pairs = dict(
        wqk=(wqkv_hbm.at[:, 0:2 * D], wqkv_ref.at[:, 0:2 * D]),
        wv=(wqkv_hbm.at[:, 2 * D:3 * D], wqkv_ref.at[:, 2 * D:3 * D]),
        win=(win_hbm, win_ref), dw1=(dw1_hbm, dw1_ref), wout=(wout_hbm, wout_ref), wo=(wo_hbm, wo_ref),
        dw2=(dw2_hbm, dw2_ref), wm=(wm_hbm, wm_ref))

    def in_copy(name):
        src, dst = pairs[name]
        return pltpu.make_async_copy(src, dst, isem.at[names.index(name)])

    def x0_copy(c):
        lo, hi = c * CK, min((c + 1) * CK, T)
        return pltpu.make_async_copy(x_hbm.at[0, lo:hi, :], x_ref.at[0, SK + lo:SK + hi, :], xsem.at[c])

    def x0_wait_full(c):
        pltpu.make_async_copy(x_ref.at[0, 0:CK, :], x_ref.at[0, 0:CK, :], xsem.at[c]).wait()

    def x1_copy():
        return pltpu.make_async_copy(x_hbm.at[1], x_ref.at[1, SK:SK + T, :], xsem.at[NC])

    def back(b, i):
        wrap = i == 0
        return jnp.where(wrap, b - 1, b), jnp.where(wrap, NQ - 1, i - 1)

    def out_start(slot, bb, ii):
        r = pl.multiple_of(ii * TQ, 16)
        rh = pl.multiple_of(jnp.where(ii > 0, r - SK, T - SK), 16)
        pltpu.make_async_copy(o_s.at[slot, 0:SK, :], o_hbm.at[bb, pl.ds(rh, SK), :], osem.at[slot]).start()
        pltpu.make_async_copy(o_s.at[slot, SK:TQ, :], o_hbm.at[bb, pl.ds(r, TQ - SK), :], osem.at[slot]).start()

    def out_wait(slot):
        pltpu.make_async_copy(o_s.at[slot], o_s.at[slot], osem.at[slot]).wait()

    def end_copy(bb):
        return pltpu.make_async_copy(oe_s, o_hbm.at[bb, T - SK:T, :], osem.at[2])

    def normalise(src, r, size, xa_dst, xa_off, v_dst):
        xn = _ln(x_ref[src, pl.ds(SK + r, size), :].astype(F32))
        xa_dst[pl.ds(xa_off + r, size), :] = xn.astype(BF16)
        v_dst[pl.ds(r, size), :] = _ones_last(xn[:, D - LANES:]).astype(BF16)

    def fold_qk():
        wqk_s[...] = (jax.lax.dot_general(wqkv_ref[:, 0:D], wqkv_ref[:, D:2 * D], NT, preferred_element_type=F32)
                      * (D ** -0.5 * LOG2E)).astype(BF16)

    def fold_vo():
        wvo = jnp.dot(wqkv_ref[:, 2 * D:3 * D], wo_ref[...], preferred_element_type=F32)
        wvo_s[...] = (wvo - wvo[D - 1:D, :]).astype(BF16)

    def publish_prev(keep):
        tail = w_s[:, TQ:TQ + HW, :]
        w_s[:, 0:HW, :] = jnp.where(keep, tail, jnp.zeros_like(tail))
        for j in range(ND):
            w_s[ND + j, HW:HW + TQ, :] = loc_s[j]
        glob = jnp.dot(on_s[...], wvo_s[...], preferred_element_type=F32)
        for j in range(ND):
            w_s[j, HW:HW + TQ, :] = glob[:, j * LANES:(j + 1) * LANES]

    def gate(h):
        return _ln(_gelu(h))

    def merge(bm, im, lo, sz, dst):
        ys = {}

        def piece(j):
            dw2 = dw2_ref[...].astype(F32)
            dw2 = dw2 + (jax.lax.broadcasted_iota(jnp.int32, dw2.shape, 0) == 2).astype(F32)
            acc = None
            for t in range(5):
                o = HW - SK + lo - 2 + t
                v = w_s[j, o:o + sz, :] * dw2[t:t + 1, j * LANES:(j + 1) * LANES]
                acc = v if acc is None else acc + v
            d = jnp.dot(acc.astype(BF16), wm_ref[j * LANES:(j + 1) * LANES, :], preferred_element_type=F32)
            ys['y'] = d if j == 0 else ys['y'] + d
            if j == 2 * ND - 1:
                xr = x_ref[bm, pl.ds(pl.multiple_of(im * TQ + lo, 16), sz), :].astype(F32)
                dst[...] = (xr + ys['y']).astype(BF16)
        return [functools.partial(piece, j) for j in range(2 * ND)]

    def sequence_end(bm):
        for task in merge(bm, NQ - 1, TQ, SK, oe_s):
            task()
        end_copy(bm).start()

    def block_tools(r):
        hs = {}

        def xa_rows(lo, size):
            return xa_s[pl.ds(r + lo, size), :]

        def carry_gate():
            for j in range(ND):
                g_s[j, 0:2 * P, :] = g_s[j, TQ:TQ + 2 * P, :]

        def loc_proj():
            hs['g'] = jnp.dot(xa_rows(2 * P, TQ), win_ref[:, D:2 * D], preferred_element_type=F32)
            hs['u'] = jnp.dot(xa_rows(P, TQ), win_ref[:, 0:D], preferred_element_type=F32)

        def loc_piece(k):
            dw1 = dw1_ref[...].astype(F32)
            g = gate(hs['g'][LB[k]:LB[k + 1]])
            for j in range(ND):
                g_s[j, 2 * P + LB[k]:2 * P + LB[k + 1], :] = g[:, j * LANES:(j + 1) * LANES]
            u = _gelu(hs['u'][LB[k]:LB[k + 1]])
            tiles = []
            for j in range(ND):
                acc = None
                for t in range(5):
                    lo = P + LB[k] - 2 + t
                    v = g_s[j, lo:lo + LB[k + 1] - LB[k], :] * dw1[t:t + 1, j * LANES:(j + 1) * LANES]
                    acc = v if acc is None else acc + v
                tiles.append((u[:, j * LANES:(j + 1) * LANES] * acc).astype(BF16))
            loc = jnp.dot(jnp.concatenate(tiles, axis=1), wout_ref[...], preferred_element_type=F32)
            for j in range(ND):
                loc_s[j, LB[k]:LB[k + 1], :] = loc[:, j * LANES:(j + 1) * LANES]

        def tail_scores():
            st = jax.lax.dot_general(z_s[...], xa_rows(P, TQ), NT, preferred_element_type=F32)
            pad = jnp.full((TQ, LANES - TK), -jnp.inf, F32)
            hs['tail'] = jnp.concatenate([st.T, pad], axis=1)

        def scores(q, c):
            if (c + 1) * CK > T:
                s = jax.lax.dot_general(q, xa_s[P + c * CK:P + T - TK, :], NT, preferred_element_type=F32)
                return jnp.concatenate([s, hs['tail']], axis=1)
            return jax.lax.dot_general(q, xa_s[P + c * CK:P + (c + 1) * CK, :], NT, preferred_element_type=F32)

        return xa_rows, carry_gate, loc_proj, loc_piece, tail_scores, scores

    def values(lo):
        return jnp.concatenate([xa_s[pl.ds(P + lo, CK), 0:D - LANES], v3_s[pl.ds(lo, CK), :]], axis=1)

    def attend(chunks, score, side, s, mrun, acc):
        for pos, c in enumerate(chunks):
            s_next = score(chunks[pos + 1]) if pos + 1 < len(chunks) else None
            mc = jnp.max(_rowmax(s), axis=-1, keepdims=True)
            mnew = mc if mrun is None else jnp.maximum(mrun, mc)
            p = jnp.exp2(s - mnew).astype(BF16)
            for task in side[pos]:
                task()
            d = jnp.dot(p, values(c * CK), preferred_element_type=F32)
            acc = d if mrun is None else acc * jnp.exp2(mrun - mnew) + d
            mrun = mnew
            s = s_next
        for task in side[len(chunks)]:
            task()
        l = acc[:, D - 1:D]
        on_s[...] = (acc * (1.0 / l)).astype(BF16)

    def step(b, i):
        xa_rows, carry_gate, loc_proj, loc_piece, tail_scores, scores = block_tools(pl.multiple_of(i * TQ, 16))

        def ln_lead():
            normalise(1, pl.multiple_of(jnp.clip((i - 1) * TS, 0, T - TS), 16), TS, xb_s, 0, vb_s)

        q = jnp.dot(xa_rows(P, TQ), wqk_s[...], preferred_element_type=F32).astype(BF16)
        carry_gate()
        side = [[] for _ in range(NC + 1)]
        for k in range(NP):
            side[LOC_SLOT[k]].append(functools.partial(loc_piece, k))
        side[0].append(loc_proj)
        side[0].append(tail_scores)
        for k, piece in enumerate(merge(*back(b, i), 0, TQ, o_s.at[i & 1])):
            side[MERGE_SLOT[k]].append(piece)
        side[0].append(ln_lead)
        attend(list(range(NC)), functools.partial(scores, q), side, scores(q, 0), None, None)

    def tail_keys():
        z_s[...] = jax.lax.dot_general(xa_s[P + T - TK:P + T, :], wqk_s[...], NT,
                                       preferred_element_type=F32).astype(BF16)

    def first_gate():
        g0 = gate(jnp.dot(xa_s[0:2 * P, :], win_ref[:, D:2 * D], preferred_element_type=F32))
        for j in range(ND):
            g_s[j, TQ:TQ + 2 * P, :] = g0[:, j * LANES:(j + 1) * LANES]

    x0_copy(0).start()
    in_copy('wqk').start()
    for c in range(1, NC):
        x0_copy(c).start()
    for name in names[1:]:
        in_copy(name).start()
    x1_copy().start()
    xa_s[0:P, :] = jnp.zeros((P, D), BF16)
    xa_s[P + T:, :] = jnp.zeros((xa_s.shape[0] - P - T, D), BF16)
    v3_s[T:TP, :] = jnp.zeros((TP - T, LANES), BF16)
    for b in range(B):
        x_ref[b, 0:SK, :] = jnp.zeros((SK, D), BF16)
    w_s[...] = jnp.zeros(w_s.shape, F32)
    acc_s[...] = jnp.zeros(acc_s.shape, F32)
    m_s[...] = jnp.full(m_s.shape, -jnp.inf, F32)

    xa_rows0, carry_gate0, loc_proj0, loc_piece0, tail_scores0, scores0 = block_tools(0)
    x0_copy(0).wait()
    in_copy('wqk').wait()
    fold_qk()
    normalise(0, 0, CK, xa_s, P, v3_s)
    q_s[...] = jnp.dot(xa_rows0(P, TQ), wqk_s[...], preferred_element_type=F32).astype(BF16)
    x0_copy(1).wait()
    s_s[0] = scores0(q_s[...], 0)
    normalise(0, CK, CK, xa_s, P, v3_s)
    NR = NC - 2

    def rolled(c, carry):
        @pl.when(c + 2 < NC - 1)
        def _():
            x0_wait_full(c + 2)

        @pl.when(c + 2 == NC - 1)
        def _():
            x0_copy(NC - 1).wait()
        s = s_s[c & 1]
        mrun = m_s[:, 0:1]
        mnew = jnp.maximum(mrun, jnp.max(_rowmax(s), axis=-1, keepdims=True))
        p = jnp.exp2(s - mnew).astype(BF16)
        k_next = xa_s[pl.ds(pl.multiple_of(P + (c + 1) * CK, 16), CK), :]
        s_s[(c + 1) & 1] = jax.lax.dot_general(q_s[...], k_next, NT, preferred_element_type=F32)
        d = jnp.dot(p, values(pl.multiple_of(c * CK, 16)), preferred_element_type=F32)
        acc_s[...] = acc_s[...] * jnp.exp2(mrun - mnew) + d
        m_s[...] = jnp.broadcast_to(mnew, m_s.shape)
        normalise(0, pl.multiple_of(jnp.minimum((c + 2) * CK, T - CK), 16), CK, xa_s, P, v3_s)
        return carry
    jax.lax.fori_loop(0, NR, rolled, 0)

    for name in names[1:]:
        in_copy(name).wait()
    tail_keys()
    tail_scores0()
    first_gate()
    carry_gate0()
    side = [[] for _ in range(3)]
    side[0] = [loc_proj0, fold_vo, functools.partial(loc_piece0, 0)]
    side[1] = [functools.partial(loc_piece0, 1), functools.partial(loc_piece0, 2)]
    side[2] = [functools.partial(loc_piece0, 3)]
    attend([NR, NR + 1], functools.partial(scores0, q_s[...]), side, s_s[NR & 1], m_s[:, 0:1], acc_s[...])
    x1_copy().wait()

    def cp_slab(j, static=False):
        r = j * TL if static else pl.multiple_of(j * TL, 16)
        xa_s[pl.ds(P + r, TL), :] = xb_s[pl.ds(r, TL), :]
        v3_s[pl.ds(r, TL), :] = vb_s[pl.ds(r, TL), :]

    def batch(b, carry):
        @pl.when(b > 0)
        def _():
            jax.lax.fori_loop(1, NL - 2, lambda j, c: cp_slab(j), None)
            cp_slab(0, True)
            cp_slab(NL - 1, True)
            tail_keys()
            first_gate()
            cp_slab(NL - 2, True)

        def main(i, c):
            n = b * NQ + i

            @pl.when(n >= 3)
            def _():
                out_wait(i & 1)
            publish_prev(i != 1)
            step(b, i)
            out_start(i & 1, *back(b, i))

            @pl.when(i == 0)
            def _():
                sequence_end(b - 1)
            return c
        jax.lax.fori_loop(jnp.where(b == 0, 1, 0), NQ, main, 0)
        return carry
    jax.lax.fori_loop(0, B, batch, 0)

    out_wait(0)
    for b in range(B - 1):
        end_copy(b).wait()
    publish_prev(True)
    r = (NQ - 1) * TQ - SK
    for lo, hi in ((0, TH), (TH, TQ)):
        for task in merge(B - 1, NQ - 1, lo, hi - lo, o_s.at[0, lo:hi, :]):
            task()
        pltpu.make_async_copy(o_s.at[0, lo:hi, :], o_hbm.at[B - 1, r + lo:r + hi, :], osem.at[0]).start()
    sequence_end(B - 1)
    out_wait(1)
    out_wait(0)
    end_copy(B - 1).wait()


@jax.jit
def pallas_standalone__conformer_family_e_branchformer__speech_kernel(
    x, w_qkv, w_att_out, w_mlp_in, dw_csgu, w_mlp_out, dw_merge, w_merge):
    B, T, D = x.shape
    TQ = 400
    NQ = T // TQ
    assert B == 2 and NQ % 2 == 0
    TP = -(-T // CK) * CK
    P = 16
    hbm = pl.BlockSpec(memory_space=pl.ANY)
    ins = (x, w_qkv, w_att_out, w_mlp_in, dw_csgu, w_mlp_out, dw_merge, w_merge)

    return pl.pallas_call(
        functools.partial(kernel, B=B, T=T, D=D, TQ=TQ, NQ=NQ, TP=TP, P=P),
        in_specs=[hbm] * len(ins),
        out_specs=hbm,
        out_shape=jax.ShapeDtypeStruct((B, T, D), x.dtype),
        scratch_shapes=[pltpu.VMEM((B, 16 + T, D), x.dtype)] + [pltpu.VMEM(a.shape, a.dtype) for a in ins[1:]] + [
            pltpu.VMEM((P + TP, D), BF16),
            pltpu.VMEM((TP, LANES), BF16),
            pltpu.VMEM((T, D), BF16),
            pltpu.VMEM((T, LANES), BF16),
            pltpu.VMEM((D, D), BF16),
            pltpu.VMEM((D, D), BF16),
            pltpu.VMEM((2 * D // LANES, TQ + 32, LANES), F32),
            pltpu.VMEM((D // LANES, TQ + 2 * P, LANES), F32),
            pltpu.VMEM((2, TQ, D), BF16),
            pltpu.VMEM((16, D), BF16),
            pltpu.VMEM((TQ, D), BF16),
            pltpu.VMEM((D // LANES, TQ, LANES), F32),
            pltpu.VMEM((T % LANES, D), BF16),
            pltpu.VMEM((TQ, D), BF16),
            pltpu.VMEM((2, TQ, CK), F32),
            pltpu.VMEM((TQ, D), F32),
            pltpu.VMEM((TQ, LANES), F32),
            pltpu.SemaphoreType.DMA((8,)),
            pltpu.SemaphoreType.DMA((TP // CK + 1,)),
            pltpu.SemaphoreType.DMA((3,)),
        ],
        compiler_params=pltpu.CompilerParams(
            vmem_limit_bytes=110 * 1024 * 1024, disable_bounds_checks=True),
    )(x, w_qkv, w_att_out, w_mlp_in, dw_csgu, w_mlp_out, dw_merge, w_merge)
```

```python
import functools
import jax
import jax.numpy as jnp
from jax.experimental import pallas as pl
from jax.experimental.pallas import tpu as pltpu

F32 = jnp.float32
BF16 = jnp.bfloat16
LOG2E = 1.4426950408889634
NT = (((1,), (1,)), ((), ()))
LANES = 128
CK = 512
LOC_ROWS = (0, 96, 208, 304, 400)
LOC_SLOT = (1, 2, 3, 4)
MERGE_SLOT = (2, 3, 4, 5, 6, 7, 8, 8)
TL = 400
TS = 448
TH = 304


def _ln(x, eps=1e-5):
    m = jnp.mean(x, axis=-1, keepdims=True)
    xc = x - m
    v = jnp.mean(xc * xc, axis=-1, keepdims=True)
    return xc * jnp.exp2(jnp.log(v + eps) * (-0.5 * LOG2E))


def _gelu(x):
    c = 0.7978845608028654
    t = x * x
    z = x * (t * (c * 0.044715) + c)
    h = 0.5 * x
    return h * jnp.tanh(z) + h


def _ones_last(xn):
    lane = jax.lax.broadcasted_iota(jnp.int32, xn.shape, 1)
    return jnp.where(lane == LANES - 1, jnp.ones_like(xn), xn)


def _rowmax(s):
    t = s[:, 0:LANES]
    for j in range(1, s.shape[1] // LANES):
        t = jnp.maximum(t, s[:, j * LANES:(j + 1) * LANES])
    return t


def kernel(x_hbm, wqkv_hbm, wo_hbm, win_hbm, dw1_hbm, wout_hbm, dw2_hbm, wm_hbm, o_hbm,
           x_ref, wqkv_ref, wo_ref, win_ref, dw1_ref, wout_ref, dw2_ref, wm_ref,
           xa_s, v3_s, xb_s, vb_s, wqk_s, wvo_s, w_s, g_s, o_s, oe_s, on_s, loc_s, z_s,
           q_s, s_s, acc_s, m_s, isem, xsem, osem,
           *, B, T, D, TQ, NQ, TP, P):
    NC = TP // CK
    ND = D // LANES
    LB = LOC_ROWS
    NP = len(LB) - 1
    NL = T // TL
    TK = T % LANES
    assert TP - T == LANES - TK
    SK = 16
    HW = SK + 8

    names = ['wqk', 'wv', 'wo', 'win', 'dw1', 'dw2', 'wout', 'wm']
    pairs = dict(
        wqk=(wqkv_hbm.at[:, 0:2 * D], wqkv_ref.at[:, 0:2 * D]),
        wv=(wqkv_hbm.at[:, 2 * D:3 * D], wqkv_ref.at[:, 2 * D:3 * D]),
        win=(win_hbm, win_ref), dw1=(dw1_hbm, dw1_ref), wout=(wout_hbm, wout_ref), wo=(wo_hbm, wo_ref),
        dw2=(dw2_hbm, dw2_ref), wm=(wm_hbm, wm_ref))

    def in_copy(name):
        src, dst = pairs[name]
        return pltpu.make_async_copy(src, dst, isem.at[names.index(name)])

    def x0_copy(c):
        lo, hi = c * CK, min((c + 1) * CK, T)
        return pltpu.make_async_copy(x_hbm.at[0, lo:hi, :], x_ref.at[0, SK + lo:SK + hi, :], xsem.at[c])

    def x0_wait_full(c):
        lo = pl.multiple_of(c * CK, 16)
        pltpu.make_async_copy(x_hbm.at[0, pl.ds(lo, CK), :], x_ref.at[0, pl.ds(SK + lo, CK), :], xsem.at[c]).wait()

    def x1_copy():
        return pltpu.make_async_copy(x_hbm.at[1], x_ref.at[1, SK:SK + T, :], xsem.at[NC])

    def back(b, i):
        wrap = i == 0
        return jnp.where(wrap, b - 1, b), jnp.where(wrap, NQ - 1, i - 1)

    def out_start(slot, bb, ii):
        r = pl.multiple_of(ii * TQ, 16)
        rh = pl.multiple_of(jnp.where(ii > 0, r - SK, T - SK), 16)
        pltpu.make_async_copy(o_s.at[slot, 0:SK, :], o_hbm.at[bb, pl.ds(rh, SK), :], osem.at[slot]).start()
        pltpu.make_async_copy(o_s.at[slot, SK:TQ, :], o_hbm.at[bb, pl.ds(r, TQ - SK), :], osem.at[slot]).start()

    def out_wait(slot):
        pltpu.make_async_copy(o_s.at[slot], o_s.at[slot], osem.at[slot]).wait()

    def end_copy(bb):
        return pltpu.make_async_copy(oe_s, o_hbm.at[bb, T - SK:T, :], osem.at[2])

    def normalise(src, r, size, xa_dst, xa_off, v_dst):
        xn = _ln(x_ref[src, pl.ds(SK + r, size), :].astype(F32))
        xa_dst[pl.ds(xa_off + r, size), :] = xn.astype(BF16)
        v_dst[pl.ds(r, size), :] = _ones_last(xn[:, D - LANES:]).astype(BF16)

    def fold_qk():
        wqk_s[...] = (jax.lax.dot_general(wqkv_ref[:, 0:D], wqkv_ref[:, D:2 * D], NT, preferred_element_type=F32)
                      * (D ** -0.5 * LOG2E)).astype(BF16)

    def fold_vo():
        wvo = jnp.dot(wqkv_ref[:, 2 * D:3 * D], wo_ref[...], preferred_element_type=F32)
        wvo_s[...] = (wvo - wvo[D - 1:D, :]).astype(BF16)

    def publish_prev(keep):
        tail = w_s[:, TQ:TQ + HW, :]
        w_s[:, 0:HW, :] = jnp.where(keep, tail, jnp.zeros_like(tail))
        for j in range(ND):
            w_s[ND + j, HW:HW + TQ, :] = loc_s[j]
        glob = jnp.dot(on_s[...], wvo_s[...], preferred_element_type=F32)
        for j in range(ND):
            w_s[j, HW:HW + TQ, :] = glob[:, j * LANES:(j + 1) * LANES]

    def gate(h):
        return _ln(_gelu(h))

    def merge(bm, im, lo, sz, dst):
        ys = {}

        def piece(j):
            dw2 = dw2_ref[...].astype(F32)
            dw2 = dw2 + (jax.lax.broadcasted_iota(jnp.int32, dw2.shape, 0) == 2).astype(F32)
            acc = None
            for t in range(5):
                o = HW - SK + lo - 2 + t
                v = w_s[j, o:o + sz, :] * dw2[t:t + 1, j * LANES:(j + 1) * LANES]
                acc = v if acc is None else acc + v
            d = jnp.dot(acc.astype(BF16), wm_ref[j * LANES:(j + 1) * LANES, :], preferred_element_type=F32)
            ys['y'] = d if j == 0 else ys['y'] + d
            if j == 2 * ND - 1:
                xr = x_ref[bm, pl.ds(pl.multiple_of(im * TQ + lo, 16), sz), :].astype(F32)
                dst[...] = (xr + ys['y']).astype(BF16)
        return [functools.partial(piece, j) for j in range(2 * ND)]

    def sequence_end(bm):
        for task in merge(bm, NQ - 1, TQ, SK, oe_s):
            task()
        end_copy(bm).start()

    def block_tools(r):
        hs = {}

        def xa_rows(lo, size):
            return xa_s[pl.ds(r + lo, size), :]

        def carry_gate():
            for j in range(ND):
                g_s[j, 0:2 * P, :] = g_s[j, TQ:TQ + 2 * P, :]

        def loc_proj():
            hs['g'] = jnp.dot(xa_rows(2 * P, TQ), win_ref[:, D:2 * D], preferred_element_type=F32)
            hs['u'] = jnp.dot(xa_rows(P, TQ), win_ref[:, 0:D], preferred_element_type=F32)

        def loc_piece(k):
            dw1 = dw1_ref[...].astype(F32)
            g = gate(hs['g'][LB[k]:LB[k + 1]])
            for j in range(ND):
                g_s[j, 2 * P + LB[k]:2 * P + LB[k + 1], :] = g[:, j * LANES:(j + 1) * LANES]
            u = _gelu(hs['u'][LB[k]:LB[k + 1]])
            tiles = []
            for j in range(ND):
                acc = None
                for t in range(5):
                    lo = P + LB[k] - 2 + t
                    v = g_s[j, lo:lo + LB[k + 1] - LB[k], :] * dw1[t:t + 1, j * LANES:(j + 1) * LANES]
                    acc = v if acc is None else acc + v
                tiles.append((u[:, j * LANES:(j + 1) * LANES] * acc).astype(BF16))
            loc = jnp.dot(jnp.concatenate(tiles, axis=1), wout_ref[...], preferred_element_type=F32)
            for j in range(ND):
                loc_s[j, LB[k]:LB[k + 1], :] = loc[:, j * LANES:(j + 1) * LANES]

        def tail_scores():
            st = jax.lax.dot_general(z_s[...], xa_rows(P, TQ), NT, preferred_element_type=F32)
            pad = jnp.full((TQ, LANES - TK), -jnp.inf, F32)
            hs['tail'] = jnp.concatenate([st.T, pad], axis=1)

        def scores(q, c):
            if (c + 1) * CK > T:
                s = jax.lax.dot_general(q, xa_s[P + c * CK:P + T - TK, :], NT, preferred_element_type=F32)
                return jnp.concatenate([s, hs['tail']], axis=1)
            return jax.lax.dot_general(q, xa_s[P + c * CK:P + (c + 1) * CK, :], NT, preferred_element_type=F32)

        return xa_rows, carry_gate, loc_proj, loc_piece, tail_scores, scores

    def values(lo):
        return jnp.concatenate([xa_s[pl.ds(P + lo, CK), 0:D - LANES], v3_s[pl.ds(lo, CK), :]], axis=1)

    def attend(chunks, score, side, s, mrun, acc):
        for pos, c in enumerate(chunks):
            s_next = score(chunks[pos + 1]) if pos + 1 < len(chunks) else None
            mc = jnp.max(_rowmax(s), axis=-1, keepdims=True)
            mnew = mc if mrun is None else jnp.maximum(mrun, mc)
            p = jnp.exp2(s - mnew).astype(BF16)
            for task in side[pos]:
                task()
            d = jnp.dot(p, values(c * CK), preferred_element_type=F32)
            acc = d if mrun is None else acc * jnp.exp2(mrun - mnew) + d
            mrun = mnew
            s = s_next
        for task in side[len(chunks)]:
            task()
        l = acc[:, D - 1:D]
        on_s[...] = (acc * (1.0 / l)).astype(BF16)

    def step(b, i):
        xa_rows, carry_gate, loc_proj, loc_piece, tail_scores, scores = block_tools(pl.multiple_of(i * TQ, 16))

        def ln_lead():
            normalise(1, pl.multiple_of(jnp.clip((i - 1) * TS, 0, T - TS), 16), TS, xb_s, 0, vb_s)

        q = jnp.dot(xa_rows(P, TQ), wqk_s[...], preferred_element_type=F32).astype(BF16)
        carry_gate()
        side = [[] for _ in range(NC + 1)]
        for k in range(NP):
            side[LOC_SLOT[k]].append(functools.partial(loc_piece, k))
        side[0].append(loc_proj)
        side[0].append(tail_scores)
        for k, piece in enumerate(merge(*back(b, i), 0, TQ, o_s.at[i & 1])):
            side[MERGE_SLOT[k]].append(piece)
        side[0].append(ln_lead)
        attend(list(range(NC)), functools.partial(scores, q), side, scores(q, 0), None, None)

    def tail_keys():
        z_s[...] = jax.lax.dot_general(xa_s[P + T - TK:P + T, :], wqk_s[...], NT,
                                       preferred_element_type=F32).astype(BF16)

    def first_gate():
        g0 = gate(jnp.dot(xa_s[0:2 * P, :], win_ref[:, D:2 * D], preferred_element_type=F32))
        for j in range(ND):
            g_s[j, TQ:TQ + 2 * P, :] = g0[:, j * LANES:(j + 1) * LANES]

    x0_copy(0).start()
    in_copy('wqk').start()
    for c in range(1, NC):
        x0_copy(c).start()
    for name in names[1:]:
        in_copy(name).start()
    x1_copy().start()
    xa_s[0:P, :] = jnp.zeros((P, D), BF16)
    xa_s[P + T:, :] = jnp.zeros((xa_s.shape[0] - P - T, D), BF16)
    v3_s[T:TP, :] = jnp.zeros((TP - T, LANES), BF16)
    for b in range(B):
        x_ref[b, 0:SK, :] = jnp.zeros((SK, D), BF16)
    w_s[:, TQ:, :] = jnp.zeros((2 * ND, w_s.shape[1] - TQ, LANES), F32)
    acc_s[...] = jnp.zeros(acc_s.shape, F32)
    m_s[...] = jnp.full(m_s.shape, -jnp.inf, F32)

    xa_rows0, carry_gate0, loc_proj0, loc_piece0, tail_scores0, scores0 = block_tools(0)
    x0_copy(0).wait()
    in_copy('wqk').wait()
    fold_qk()
    normalise(0, 0, CK, xa_s, P, v3_s)
    q_s[...] = jnp.dot(xa_rows0(P, TQ), wqk_s[...], preferred_element_type=F32).astype(BF16)
    x0_copy(1).wait()
    s_s[0] = scores0(q_s[...], 0)
    normalise(0, CK, CK, xa_s, P, v3_s)
    NR = NC - 2

    def rolled(c, carry):
        @pl.when(c + 2 < NC - 1)
        def _():
            x0_wait_full(c + 2)

        @pl.when(c + 2 == NC - 1)
        def _():
            x0_copy(NC - 1).wait()
        s = s_s[c & 1]
        mrun = m_s[:, 0:1]
        mnew = jnp.maximum(mrun, jnp.max(_rowmax(s), axis=-1, keepdims=True))
        p = jnp.exp2(s - mnew).astype(BF16)
        k_next = xa_s[pl.ds(pl.multiple_of(P + (c + 1) * CK, 16), CK), :]
        s_s[(c + 1) & 1] = jax.lax.dot_general(q_s[...], k_next, NT, preferred_element_type=F32)
        d = jnp.dot(p, values(pl.multiple_of(c * CK, 16)), preferred_element_type=F32)
        acc_s[...] = acc_s[...] * jnp.exp2(mrun - mnew) + d
        m_s[...] = jnp.broadcast_to(mnew, m_s.shape)
        normalise(0, pl.multiple_of(jnp.minimum((c + 2) * CK, T - CK), 16), CK, xa_s, P, v3_s)
        return carry
    jax.lax.fori_loop(0, NR, rolled, 0)

    for name in names[1:]:
        in_copy(name).wait()
    tail_keys()
    first_gate()
    loc_proj0()
    tail_scores0()
    carry_gate0()
    piece = [functools.partial(loc_piece0, k) for k in range(NP)]
    side = [piece[0:2], [fold_vo, piece[2]], piece[3:]]
    attend([NR, NR + 1], functools.partial(scores0, q_s[...]), side, s_s[NR & 1], m_s[:, 0:1], acc_s[...])
    x1_copy().wait()

    def cp_slab(j, static=False):
        r = j * TL if static else pl.multiple_of(j * TL, 16)
        xa_s[pl.ds(P + r, TL), :] = xb_s[pl.ds(r, TL), :]
        v3_s[pl.ds(r, TL), :] = vb_s[pl.ds(r, TL), :]

    def batch(b, carry):
        @pl.when(b > 0)
        def _():
            jax.lax.fori_loop(1, NL - 2, lambda j, c: cp_slab(j), None)
            cp_slab(0, True)
            cp_slab(NL - 1, True)
            tail_keys()
            first_gate()
            cp_slab(NL - 2, True)

        def main(i, c):
            n = b * NQ + i

            @pl.when(n >= 3)
            def _():
                out_wait(i & 1)
            publish_prev(i != 1)
            step(b, i)
            out_start(i & 1, *back(b, i))

            @pl.when(i == 0)
            def _():
                sequence_end(b - 1)
            return c
        jax.lax.fori_loop(jnp.where(b == 0, 1, 0), NQ, main, 0)
        return carry
    jax.lax.fori_loop(0, B, batch, 0)

    out_wait(0)
    for b in range(B - 1):
        end_copy(b).wait()
    publish_prev(True)
    r = (NQ - 1) * TQ - SK
    for lo, hi in ((0, TH), (TH, TQ)):
        for task in merge(B - 1, NQ - 1, lo, hi - lo, o_s.at[0, lo:hi, :]):
            task()
        pltpu.make_async_copy(o_s.at[0, lo:hi, :], o_hbm.at[B - 1, r + lo:r + hi, :], osem.at[0]).start()
    sequence_end(B - 1)
    out_wait(1)
    out_wait(0)
    end_copy(B - 1).wait()


@jax.jit
def pallas_standalone__conformer_family_e_branchformer__speech_kernel(
    x, w_qkv, w_att_out, w_mlp_in, dw_csgu, w_mlp_out, dw_merge, w_merge):
    B, T, D = x.shape
    TQ = 400
    NQ = T // TQ
    assert B == 2 and NQ % 2 == 0
    TP = -(-T // CK) * CK
    P = 16
    hbm = pl.BlockSpec(memory_space=pl.ANY)
    ins = (x, w_qkv, w_att_out, w_mlp_in, dw_csgu, w_mlp_out, dw_merge, w_merge)

    return pl.pallas_call(
        functools.partial(kernel, B=B, T=T, D=D, TQ=TQ, NQ=NQ, TP=TP, P=P),
        in_specs=[hbm] * len(ins),
        out_specs=hbm,
        out_shape=jax.ShapeDtypeStruct((B, T, D), x.dtype),
        scratch_shapes=[pltpu.VMEM((B, 16 + T, D), x.dtype)] + [pltpu.VMEM(a.shape, a.dtype) for a in ins[1:]] + [
            pltpu.VMEM((P + TP, D), BF16),
            pltpu.VMEM((TP, LANES), BF16),
            pltpu.VMEM((T, D), BF16),
            pltpu.VMEM((T, LANES), BF16),
            pltpu.VMEM((D, D), BF16),
            pltpu.VMEM((D, D), BF16),
            pltpu.VMEM((2 * D // LANES, TQ + 32, LANES), F32),
            pltpu.VMEM((D // LANES, TQ + 2 * P, LANES), F32),
            pltpu.VMEM((2, TQ, D), BF16),
            pltpu.VMEM((16, D), BF16),
            pltpu.VMEM((TQ, D), BF16),
            pltpu.VMEM((D // LANES, TQ, LANES), F32),
            pltpu.VMEM((T % LANES, D), BF16),
            pltpu.VMEM((TQ, D), BF16),
            pltpu.VMEM((2, TQ, CK), F32),
            pltpu.VMEM((TQ, D), F32),
            pltpu.VMEM((TQ, LANES), F32),
            pltpu.SemaphoreType.DMA((8,)),
            pltpu.SemaphoreType.DMA((TP // CK + 1,)),
            pltpu.SemaphoreType.DMA((3,)),
        ],
        compiler_params=pltpu.CompilerParams(
            vmem_limit_bytes=110 * 1024 * 1024, disable_bounds_checks=True),
    )(x, w_qkv, w_att_out, w_mlp_in, dw_csgu, w_mlp_out, dw_merge, w_merge)
```
